```python
import jax
import jax.numpy as jnp

def _softmax(x, axis=-1):
    return jax.nn.softmax(x, axis=axis)
def _gelu(x):
    return jax.nn.gelu(x, approximate=True)
def _silu(x):
    return jax.nn.silu(x)
def _sigmoid(x):
    return jax.nn.sigmoid(x)
def _layernorm(x, axis=-1, eps=1e-5):
    m = jnp.mean(x, axis=axis, keepdims=True)
    v = jnp.var(x, axis=axis, keepdims=True)
    return (x - m) / jnp.sqrt(v + eps)
def _scatter_add(tgt, idx, src, axis=0):
    return tgt.at[idx].add(src)
def _segment_sum(src, seg, n):
    return jax.ops.segment_sum(src, seg, n)
class _Rng:
    def __init__(self, key):
        self._k = key
    def _next(self):
        self._k, sub = jax.random.split(self._k)
        return sub
    def normal(self, shape):
        return jax.random.normal(self._next(), shape, dtype=jnp.bfloat16)
    def randint(self, lo, hi, shape):
        return jax.random.randint(self._next(), shape, lo, hi, dtype=jnp.int32)
    def uniform(self, shape, lo=0.0, hi=1.0):
        return jax.random.uniform(self._next(), shape, jnp.bfloat16, lo, hi)
    def permutation(self, n):
        return jax.random.permutation(self._next(), n)


kernel_name = 'interleave_layers__sliding_block_cached__glu_gated_swiglu__decode'

def setup_inputs():
    _rng = _Rng(jax.random.key(int.from_bytes(__import__("os").urandom(4), "little")))
    _w = (lambda a: (lambda t: t.astype(jnp.bfloat16) if jnp.issubdtype(t.dtype, jnp.floating) else t)(jnp.asarray(a)))
    def _A_setup():
        B, Sq, D = 1, 1, 640
        Hq, Hkv, Sk, Dh = 32, 32, 32768, 192
        assert Hq % Hkv == 0, (Hq, Hkv)
        return {
            "x": _w((lambda *s: _rng.normal(s) * 0.05)(B, Sq, D)),
            "k_cache": _w((lambda *s: _rng.normal(s) * 0.05)(B, Hkv, Sk, Dh)),
            "v_cache": _w((lambda *s: _rng.normal(s) * 0.05)(B, Hkv, Sk, Dh)),
            "wq": _w((lambda *s: _rng.normal(s) * 0.05)(D, Hq * Dh) * (D ** -0.5)),
            "wo": _w((lambda *s: _rng.normal(s) * 0.05)(Hq * Dh, D) * ((Hq * Dh) ** -0.5)),
        }
    _A_in = _A_setup()

    def _B_setup():
        B, S, D, F = 1, 1, 640, 1536
        return {
            "x": _w((lambda *s: _rng.normal(s) * 0.05)(B, S, D)),
            "w1": _w((lambda *s: _rng.normal(s) * 0.05)(D, F) * (2.0 / D) ** 0.5),
            "w3": _w((lambda *s: _rng.normal(s) * 0.05)(D, F) * (2.0 / D) ** 0.5),
            "w2": _w((lambda *s: _rng.normal(s) * 0.05)(F, D) * (2.0 / F) ** 0.5),
        }
    _B_in = _B_setup()

    return {
        "A_x": _A_in["x"],
        "A_k_cache": _A_in["k_cache"],
        "A_v_cache": _A_in["v_cache"],
        "A_wq": _A_in["wq"],
        "A_wo": _A_in["wo"],
        "B_x": _B_in["x"],
        "B_w1": _B_in["w1"],
        "B_w3": _B_in["w3"],
        "B_w2": _B_in["w2"],
    }

def reference(A_x, A_k_cache, A_v_cache, A_wq, A_wo, B_x, B_w1, B_w3, B_w2):
    def _A_ref(x, k_cache, v_cache, wq, wo):
        B, Sq, D = x.shape
        Hq, Dh = 32, 192
        Hkv, Sk = k_cache.shape[1], k_cache.shape[2]
        W = min(4096, max(256, Sk // 4))
        rep = Hq // Hkv
        q = (lambda x, *d: x.transpose(*d))((x @ wq).reshape(B, Sq, Hq, Dh), 0, 2, 1, 3)
        k = jnp.repeat(k_cache[:, :, Sk - W:, :], rep, axis=1)
        v = jnp.repeat(v_cache[:, :, Sk - W:, :], rep, axis=1)
        scores = jnp.einsum("bhqd,bhkd->bhqk", q, k) * (Dh ** -0.5)
        p = _softmax(scores, axis=-1)
        o = jnp.einsum("bhqk,bhkd->bhqd", p, v)
        return (lambda x, *d: x.transpose(*d))(o, 0, 2, 1, 3).reshape(B, Sq, Hq * Dh) @ wo

    def _B_ref(x, w1, w3, w2):
        gate = jnp.einsum("bsd,df->bsf", x, w1)
        up = jnp.einsum("bsd,df->bsf", x, w3)
        h = _silu(gate) * up
        out = jnp.einsum("bsf,fd->bsd", h, w2)
        return out

    x = A_x
    x = x + _A_ref(_layernorm(x, axis=-1), A_k_cache, A_v_cache, A_wq, A_wo)
    x = x + _B_ref(_layernorm(x, axis=-1), B_w1, B_w3, B_w2)
    x = x + _A_ref(_layernorm(x, axis=-1), A_k_cache, A_v_cache, A_wq, A_wo)
    x = x + _B_ref(_layernorm(x, axis=-1), B_w1, B_w3, B_w2)
    return x
```

```python
import jax
import jax.numpy as jnp
from jax import lax
import jax.experimental.pallas as pl
import jax.experimental.pallas.tpu as pltpu

BF16 = jnp.bfloat16
F32 = jnp.float32
U32 = jnp.uint32

HQ, DH = 32, 192
LANES = 128
HG = 8
NG = HQ // HG
GR = HG * DH
EPS = 1e-5


def _layernorm(x):
    m = jnp.mean(x, axis=-1, keepdims=True)
    c = x - m
    v = jnp.mean(c * c, axis=-1, keepdims=True)
    return c / jnp.sqrt(v + EPS)


def _rnd(x):
    return x.astype(BF16).astype(F32)


def _make_kernel(D, F, SK, W):
    NJ = W // LANES
    ND = D // LANES
    scale = DH ** -0.5

    def kernel(x_hbm, k_hbm, v_hbm, wq_hbm, wo_hbm, w1_hbm, w3_hbm, w2_hbm, o_ref,
               xb, kb, vb, wq, wo, w1, w3, w2, qbd, s_ref, p_ref, acc_ref,
               sem_k, sem_v, sem_w):
        def k_copy(j):
            return pltpu.make_async_copy(
                k_hbm.at[:, pl.ds(SK - W + j * LANES, LANES)], kb.at[j], sem_k.at[j])

        def v_copy(j):
            return pltpu.make_async_copy(
                v_hbm.at[:, pl.ds(SK - W + j * LANES, LANES)], vb.at[j], sem_v.at[j])

        x_copy = pltpu.make_async_copy(x_hbm, xb, sem_w.at[0])
        wq_copy = pltpu.make_async_copy(wq_hbm, wq, sem_w.at[1])
        w1_copy = pltpu.make_async_copy(w1_hbm, w1, sem_w.at[2])
        w3_copy = pltpu.make_async_copy(w3_hbm, w3, sem_w.at[3])
        wo_copy = [pltpu.make_async_copy(wo_hbm.at[:, pl.ds(c * LANES, LANES)], wo.at[c],
                                         sem_w.at[4 + c]) for c in range(ND)]
        w2_copy = [pltpu.make_async_copy(w2_hbm.at[:, pl.ds(c * LANES, LANES)], w2.at[c],
                                         sem_w.at[4 + ND + c]) for c in range(ND)]

        x_copy.start()
        wq_copy.start()
        for j in range(NJ):
            k_copy(j).start()
        for j in range(NJ):
            v_copy(j).start()
        for c in wo_copy:
            c.start()
        w1_copy.start()
        w3_copy.start()
        for c in w2_copy:
            c.start()

        kbu = kb.bitcast(U32)
        vbu = vb.bitcast(U32)
        wou = wo.bitcast(U32)
        w2u = w2.bitcast(U32)

        row = lax.broadcasted_iota(jnp.int32, (2 * HG, GR), 0)
        col = lax.broadcasted_iota(jnp.int32, (2 * HG, GR), 1)
        diag = (col >= row * DH) & (col < (row + 1) * DH)

        def attention(x, first):
            h = jnp.broadcast_to(_layernorm(x), (2 * HG, D)).astype(BF16)
            if first:
                wq_copy.wait()
            for g in range(NG):
                q = jnp.dot(h, wq[:, g * GR:(g + 1) * GR], preferred_element_type=F32)
                qbd[g] = jnp.where(diag, q, 0.0).astype(BF16)

            def qk(j, carry):
                if first:
                    k_copy(j).wait()
                for g in range(NG):
                    kt = pltpu.bitcast(kbu[j, g * GR // 2:(g + 1) * GR // 2, :], BF16)
                    s = jnp.dot(qbd[g], kt, preferred_element_type=F32)[0:HG]
                    s_ref[g, j] = s * scale
                return carry

            lax.fori_loop(0, NJ, qk, 0, unroll=1 if first else 4)

            inv = []
            for g in range(NG):
                s = s_ref[g]
                m = jnp.max(jnp.max(s, axis=0), axis=-1, keepdims=True)
                e = jnp.exp(s - m[None])
                l = jnp.sum(jnp.sum(e, axis=0), axis=-1, keepdims=True)
                inv.append(1.0 / l)
                p_ref[g] = jnp.concatenate([e, jnp.zeros_like(e)], axis=1).astype(BF16)

            acc_ref[...] = jnp.zeros_like(acc_ref)

            def pv(j, carry):
                if first:
                    v_copy(j).wait()
                for g in range(NG):
                    vt = pltpu.bitcast(vbu[j, g * GR // 2:(g + 1) * GR // 2, :], BF16)
                    o = lax.dot_general(p_ref[g, j], vt, (((1,), (1,)), ((), ())),
                                        preferred_element_type=F32)
                    acc_ref[g] += o[0:HG]
                return carry

            lax.fori_loop(0, NJ, pv, 0)

            obd = []
            for g in range(NG):
                o = jnp.where(diag[0:HG], acc_ref[g] * inv[g], 0.0)
                obd.append(jnp.concatenate([o, jnp.zeros_like(o)], axis=0).astype(BF16))
            obd = jnp.concatenate(obd, axis=1)
            outs = []
            for c in range(ND):
                if first:
                    wo_copy[c].wait()
                y = jnp.dot(obd, pltpu.bitcast(wou[c], BF16), preferred_element_type=F32)
                outs.append(jnp.sum(y[0:HG], axis=0, keepdims=True))
            return jnp.concatenate(outs, axis=1)

        def ffn(x, first):
            h = jnp.broadcast_to(_layernorm(x), (2 * HG, D)).astype(BF16)
            if first:
                w1_copy.wait()
            gate = jnp.dot(h, w1[...], preferred_element_type=F32)
            if first:
                w3_copy.wait()
            up = jnp.dot(h, w3[...], preferred_element_type=F32)
            a = (gate * jax.nn.sigmoid(gate) * up).astype(BF16)
            outs = []
            for c in range(ND):
                if first:
                    w2_copy[c].wait()
                y = jnp.dot(a, pltpu.bitcast(w2u[c], BF16), preferred_element_type=F32)
                outs.append(y[0:1])
            return jnp.concatenate(outs, axis=1)

        x_copy.wait()
        x = xb[...].astype(F32)
        for first in (True, False):
            x = _rnd(x + _rnd(attention(x, first)))
            x = _rnd(x + _rnd(ffn(x, first)))
        o_ref[...] = x.astype(o_ref.dtype)

    return kernel


@jax.jit
def pallas_interleave_layers__sliding_block_cached__glu_gated_swiglu__decode_kernel(
    A_x: jax.Array,
    A_k_cache: jax.Array,
    A_v_cache: jax.Array,
    A_wq: jax.Array,
    A_wo: jax.Array,
    B_x: jax.Array,
    B_w1: jax.Array,
    B_w3: jax.Array,
    B_w2: jax.Array,
):
    del B_x
    D = A_x.shape[-1]
    F = B_w1.shape[-1]
    SK = A_k_cache.shape[2]
    W = min(4096, max(256, SK // 4))
    R = HQ * DH
    NJ = W // LANES
    ND = D // LANES

    k_t = jnp.swapaxes(A_k_cache[0], 1, 2).reshape(R, SK)
    v_t = jnp.swapaxes(A_v_cache[0], 1, 2).reshape(R, SK)

    hbm = pl.BlockSpec(memory_space=pl.ANY)
    out = pl.pallas_call(
        _make_kernel(D, F, SK, W),
        out_shape=jax.ShapeDtypeStruct((1, D), A_x.dtype),
        in_specs=[hbm] * 8,
        out_specs=pl.BlockSpec(memory_space=pltpu.VMEM),
        scratch_shapes=[
            pltpu.VMEM((1, D), BF16),
            pltpu.VMEM((NJ, R, LANES), BF16),
            pltpu.VMEM((NJ, R, LANES), BF16),
            pltpu.VMEM((D, R), BF16),
            pltpu.VMEM((ND, R, LANES), BF16),
            pltpu.VMEM((D, F), BF16),
            pltpu.VMEM((D, F), BF16),
            pltpu.VMEM((ND, F, LANES), BF16),
            pltpu.VMEM((NG, 2 * HG, GR), BF16),
            pltpu.VMEM((NG, NJ, HG, LANES), F32),
            pltpu.VMEM((NG, NJ, 2 * HG, LANES), BF16),
            pltpu.VMEM((NG, HG, GR), F32),
            pltpu.SemaphoreType.DMA((NJ,)),
            pltpu.SemaphoreType.DMA((NJ,)),
            pltpu.SemaphoreType.DMA((4 + 2 * ND,)),
        ],
        compiler_params=pltpu.CompilerParams(vmem_limit_bytes=127 * 1024 * 1024),
    )(A_x.reshape(1, D), k_t, v_t, A_wq, A_wo, B_w1, B_w3, B_w2)
    return out.reshape(A_x.shape)
```

```python
import jax
import jax.numpy as jnp
from jax import lax
import jax.experimental.pallas as pl
import jax.experimental.pallas.tpu as pltpu

BF16 = jnp.bfloat16
F32 = jnp.float32
U32 = jnp.uint32

HQ, DH = 32, 192
LANES = 128
HG = 8
NG = HQ // HG
GR = HG * DH
PR = 2 * DH
EPS = 1e-5
AHEAD = 3
NMG = 4
NPAIR = (NG - NMG) * HG // 2
IB = 2
QK_M_AFTER = 9
LOG2E = 1.4426950408889634


def _layernorm(x):
    m = jnp.mean(x, axis=-1, keepdims=True)
    c = x - m
    v = jnp.mean(c * c, axis=-1, keepdims=True)
    return c / jnp.sqrt(v + EPS)


def _rnd(x):
    return x.astype(BF16).astype(F32)


def _bf(u):
    return pltpu.bitcast(u, BF16)


def _make_kernel(D, F, SK, W):
    NJ = W // LANES
    ND = D // LANES
    cexp = DH ** -0.5 * LOG2E

    def kernel(x_hbm, k_hbm, v_hbm, wq_hbm, wo_hbm, w1_hbm, w3_hbm, w2_hbm, o_ref,
               xb, kb, vb, wq, wo, w1, w3, w2, qbd, s_ref, p_ref, acc_ref, pm_ref, pp_ref,
               sem_k, sem_v, sem_w):
        def k_copy(j):
            return pltpu.make_async_copy(
                k_hbm.at[:, pl.ds(SK - W + j * LANES, LANES)], kb.at[j], sem_k.at[j])

        def v_copy(j):
            return pltpu.make_async_copy(
                v_hbm.at[:, pl.ds(SK - W + j * LANES, LANES)], vb.at[j], sem_v.at[j])

        x_copy = pltpu.make_async_copy(x_hbm, xb, sem_w.at[0])
        wq_copy = pltpu.make_async_copy(wq_hbm, wq, sem_w.at[1])
        w1_copy = pltpu.make_async_copy(w1_hbm, w1, sem_w.at[2])
        w3_copy = pltpu.make_async_copy(w3_hbm, w3, sem_w.at[3])
        wo_copy = [pltpu.make_async_copy(wo_hbm.at[:, pl.ds(c * LANES, LANES)], wo.at[c],
                                         sem_w.at[4 + c]) for c in range(ND)]
        w2_copy = [pltpu.make_async_copy(w2_hbm.at[:, pl.ds(c * LANES, LANES)], w2.at[c],
                                         sem_w.at[4 + ND + c]) for c in range(ND)]

        tail = wo_copy + [w1_copy, w3_copy] + w2_copy
        x_copy.start()
        wq_copy.start()
        for j in range(AHEAD):
            k_copy(j).start()

        kbu = kb.bitcast(U32)
        vbu = vb.bitcast(U32)
        wou = wo.bitcast(U32)
        w2u = w2.bitcast(U32)

        row = lax.broadcasted_iota(jnp.int32, (2 * HG, GR), 0)
        col = lax.broadcasted_iota(jnp.int32, (2 * HG, GR), 1)
        diag = (col >= row * DH) & (col < (row + 1) * DH)

        sub = lax.broadcasted_iota(jnp.int32, (8, PR), 0)
        lane = lax.broadcasted_iota(jnp.int32, (8, PR), 1)
        half = jnp.where(lane < DH, jnp.uint32(0x0000FFFF), jnp.uint32(0xFFFF0000))
        for ph in range(4):
            pm_ref[ph] = jnp.where(sub == ph, half, jnp.uint32(0))

        def group_q(h, g):
            q = jnp.dot(h, wq[:, g * GR:(g + 1) * GR], preferred_element_type=F32)
            qbd[g] = pltpu.bitcast(jnp.where(diag, q, 0.0).astype(BF16), U32)

        def group_qk(g, j):
            kt = _bf(kbu[j, g * GR // 2:(g + 1) * GR // 2, :])
            s_ref[g, j] = jnp.dot(_bf(qbd[g]), kt, preferred_element_type=F32)[0:HG]

        def group_softmax(g):
            s = s_ref[g]
            m = jnp.max(jnp.max(s, axis=0), axis=-1, keepdims=True)
            e = jnp.exp2((s - m[None]) * cexp)
            l = jnp.sum(jnp.sum(e, axis=0), axis=-1, keepdims=True)
            p_ref[g] = pltpu.bitcast(
                jnp.concatenate([e, jnp.zeros_like(e)], axis=1).astype(BF16), U32)
            return 1.0 / l

        def masked_o(o, inv):
            o = jnp.where(diag[0:HG], o * inv, 0.0)
            return jnp.concatenate([o, jnp.zeros_like(o)], axis=0).astype(BF16)

        def attention1(x):
            h = jnp.broadcast_to(_layernorm(x), (2 * HG, D)).astype(BF16)
            wq_copy.wait()
            for g in range(NG):
                group_q(h, g)

            def qk(j, carry):
                k_copy(j).wait()

                @pl.when(j + AHEAD < NJ)
                def _():
                    k_copy(j + AHEAD).start()

                @pl.when(j + AHEAD >= NJ)
                def _():
                    v_copy(j + AHEAD - NJ).start()

                for g in range(NG):
                    group_qk(g, j)
                return carry

            lax.fori_loop(0, NJ, qk, 0)
            inv = [group_softmax(g) for g in range(NG)]
            acc_ref[...] = jnp.zeros_like(acc_ref)

            def pv(j, carry):
                v_copy(j).wait()

                @pl.when(j + AHEAD < NJ)
                def _():
                    v_copy(j + AHEAD).start()

                @pl.when(j + AHEAD == NJ)
                def _():
                    for c in tail:
                        c.start()

                for g in range(NG):
                    vt = _bf(vbu[j, g * GR // 2:(g + 1) * GR // 2, :])
                    o = lax.dot_general(_bf(p_ref[g, j]), vt, (((1,), (1,)), ((), ())),
                                        preferred_element_type=F32)
                    acc_ref[g] += o[0:HG]
                    if g >= NG - NMG:
                        for t in range(GR // LANES):
                            tile = vt[t * LANES:(t + 1) * LANES]
                            r0 = (g * GR + t * LANES) // 2
                            vbu[j, r0:r0 + LANES // 2, :] = pltpu.bitcast(tile.T, U32)
                return carry

            lax.fori_loop(0, NJ, pv, 0)

            obd = jnp.concatenate([masked_o(acc_ref[g], inv[g]) for g in range(NG)], axis=1)
            outs = []
            for c in range(ND):
                wo_copy[c].wait()
                y = jnp.dot(obd, _bf(wou[c]), preferred_element_type=F32)
                outs.append(jnp.sum(y[0:HG], axis=0, keepdims=True))
            return jnp.concatenate(outs, axis=1)

        def attention2(x):
            h = jnp.broadcast_to(_layernorm(x), (2 * HG, D)).astype(BF16)
            out = [None] * ND

            def accumulate(c, y):
                out[c] = y if out[c] is None else out[c] + y

            def pair_scores(p):
                q = jnp.dot(h, wq[:, p * PR:(p + 1) * PR], preferred_element_type=F32)
                qu = pltpu.bitcast(q.astype(BF16), U32)
                lhs = jnp.concatenate([_bf(qu & pm_ref[ph]) for ph in range(4)], axis=1)
                ss = []
                for jo in range(NJ // 4):
                    kt = jnp.concatenate(
                        [_bf(kbu[4 * jo + ph, p * PR // 2:(p + 1) * PR // 2, :]) for ph in range(4)],
                        axis=0)
                    ss.append(jnp.dot(lhs, kt, preferred_element_type=F32)[0:8])
                m = ss[0]
                for s in ss[1:]:
                    m = jnp.maximum(m, s)
                m = jnp.maximum(m, pltpu.roll(m, 4, 0))
                m = jnp.maximum(m, pltpu.roll(m, 2, 0))
                m = jnp.max(m, axis=-1, keepdims=True)
                l = None
                for jo, s in enumerate(ss):
                    e = jnp.exp2((s - m) * cexp)
                    pp_ref[p, jo] = e
                    l = e if l is None else l + e
                l = l + pltpu.roll(l, 4, 0)
                l = l + pltpu.roll(l, 2, 0)
                return 1.0 / jnp.sum(l, axis=-1, keepdims=True)

            def pair_values(p, inv):
                for hd in range(2):
                    scale = jnp.broadcast_to(inv[hd:hd + 1], (8, 1))
                    for blk in range(DH // (16 * IB)):
                        r0 = p * PR + hd * DH + blk * 16 * IB
                        accs = [None] * (2 * IB)
                        for j in range(NJ):
                            sl = 2 * (j % 4) + hd
                            pj = jnp.broadcast_to(pp_ref[p, j // 4, sl:sl + 1, :], (8, LANES))
                            vf = vb[j, r0:r0 + 16 * IB, :].astype(F32)
                            for a in range(2 * IB):
                                t = vf[8 * a:8 * a + 8] * pj
                                accs[a] = t if accs[a] is None else accs[a] + t
                        os_ = [_rnd(jnp.sum(a, axis=-1, keepdims=True) * scale) for a in accs]
                        for c in range(ND):
                            wf = wo[c, r0:r0 + 16 * IB, :].astype(F32)
                            y = None
                            for a in range(2 * IB):
                                t = wf[8 * a:8 * a + 8] * os_[a]
                                y = t if y is None else y + t
                            accumulate(c, y)

            def group_values(g, inv):
                pg = jnp.concatenate([_bf(p_ref[g, j]) for j in range(NJ)], axis=1)
                os_ = []
                for t in range(GR // LANES):
                    r0 = (g * GR + t * LANES) // 2
                    vt = jnp.concatenate(
                        [_bf(vbu[j, r0:r0 + LANES // 2, :]) for j in range(NJ)], axis=0)
                    os_.append(jnp.dot(pg, vt, preferred_element_type=F32)[0:HG])
                ob = masked_o(jnp.concatenate(os_, axis=1), inv)
                for c in range(ND):
                    y = jnp.dot(ob, _bf(wou[c, g * GR // 2:(g + 1) * GR // 2, :]),
                                preferred_element_type=F32)
                    accumulate(c, y[0:HG])

            ginv = {}

            def mxu_group_scores():
                for g in range(NG - NMG, NG):
                    group_q(h, g)
                    for j in range(NJ):
                        group_qk(g, j)
                    ginv[g] = group_softmax(g)

            invs = {}
            if NPAIR:
                invs[0] = pair_scores(0)
            for p in range(NPAIR):
                if p + 1 == QK_M_AFTER:
                    mxu_group_scores()
                if p + 1 < NPAIR:
                    invs[p + 1] = pair_scores(p + 1)
                pair_values(p, invs[p])
            if not ginv:
                mxu_group_scores()
            for g in range(NG - NMG, NG):
                group_values(g, ginv[g])
            return jnp.concatenate([jnp.sum(y, axis=0, keepdims=True) for y in out], axis=1)

        def ffn(x, first):
            h = jnp.broadcast_to(_layernorm(x), (2 * HG, D)).astype(BF16)
            if first:
                w1_copy.wait()
            gate = jnp.dot(h, w1[...], preferred_element_type=F32)
            if first:
                w3_copy.wait()
            up = jnp.dot(h, w3[...], preferred_element_type=F32)
            a = (gate * jax.nn.sigmoid(gate) * up).astype(BF16)
            outs = []
            for c in range(ND):
                if first:
                    w2_copy[c].wait()
                y = jnp.dot(a, _bf(w2u[c]), preferred_element_type=F32)
                outs.append(y[0:1])
            return jnp.concatenate(outs, axis=1)

        x_copy.wait()
        x = xb[...].astype(F32)
        x = _rnd(x + _rnd(attention1(x)))
        x = _rnd(x + _rnd(ffn(x, True)))
        x = _rnd(x + _rnd(attention2(x)))
        x = _rnd(x + _rnd(ffn(x, False)))
        o_ref[...] = x.astype(o_ref.dtype)

    return kernel


@jax.jit
def pallas_interleave_layers__sliding_block_cached__glu_gated_swiglu__decode_kernel(
    A_x, A_k_cache, A_v_cache, A_wq, A_wo, B_x, B_w1, B_w3, B_w2,
):
    del B_x
    D = A_x.shape[-1]
    F = B_w1.shape[-1]
    SK = A_k_cache.shape[2]
    W = min(4096, max(256, SK // 4))
    R = HQ * DH
    NJ = W // LANES
    ND = D // LANES

    k_t = jnp.swapaxes(A_k_cache[0], 1, 2).reshape(R, SK)
    v_t = jnp.swapaxes(A_v_cache[0], 1, 2).reshape(R, SK)

    hbm = pl.BlockSpec(memory_space=pl.ANY)
    out = pl.pallas_call(
        _make_kernel(D, F, SK, W),
        out_shape=jax.ShapeDtypeStruct((1, D), A_x.dtype),
        in_specs=[hbm] * 8,
        out_specs=pl.BlockSpec(memory_space=pltpu.VMEM),
        scratch_shapes=[
            pltpu.VMEM((1, D), BF16),
            pltpu.VMEM((NJ, R, LANES), BF16),
            pltpu.VMEM((NJ, R, LANES), BF16),
            pltpu.VMEM((D, R), BF16),
            pltpu.VMEM((ND, R, LANES), BF16),
            pltpu.VMEM((D, F), BF16),
            pltpu.VMEM((D, F), BF16),
            pltpu.VMEM((ND, F, LANES), BF16),
            pltpu.VMEM((NG, HG, GR), U32),
            pltpu.VMEM((NG, NJ, HG, LANES), F32),
            pltpu.VMEM((NG, NJ, HG, LANES), U32),
            pltpu.VMEM((NG, HG, GR), F32),
            pltpu.VMEM((4, 8, PR), U32),
            pltpu.VMEM((max(NPAIR, 1), NJ // 4, 8, LANES), F32),
            pltpu.SemaphoreType.DMA((NJ,)),
            pltpu.SemaphoreType.DMA((NJ,)),
            pltpu.SemaphoreType.DMA((4 + 2 * ND,)),
        ],
        compiler_params=pltpu.CompilerParams(vmem_limit_bytes=127 * 1024 * 1024),
    )(A_x.reshape(1, D), k_t, v_t, A_wq, A_wo, B_w1, B_w3, B_w2)
    return out.reshape(A_x.shape)
```

```python
import jax
import jax.numpy as jnp
from jax import lax
import jax.experimental.pallas as pl
import jax.experimental.pallas.tpu as pltpu

BF16 = jnp.bfloat16
F32 = jnp.float32
U32 = jnp.uint32

HQ, DH = 32, 192
R = HQ * DH
LANES = 128
HG = 8
NG = HQ // HG
GR = HG * DH
NP = HQ // 2
PR = 2 * DH
PT = PR // LANES
EPS = 1e-5
LOG2E = 1.4426950408889634

PRIO = 0
AHEAD = 4
QC = 512
NV = 11
IB = 2
PVS = 2
Q_AHEAD = 2
SOFTMAX_LAT = 400
MXU_TILE = 85
MXU_LAT = 100
VPU_BLOCK = 133
VPU_LAT = 150
TIE_EVERY = 1
WO_AT = 20
DM_AT = 24
NOCSE = 1


def _layernorm(x):
    m = jnp.mean(x, axis=-1, keepdims=True)
    c = x - m
    v = jnp.mean(c * c, axis=-1, keepdims=True)
    return c / jnp.sqrt(v + EPS)


def _rnd(x):
    return x.astype(BF16).astype(F32)


def _bf(u):
    return pltpu.bitcast(u, BF16)


def _pack(x):
    return pltpu.bitcast(jnp.concatenate([x, jnp.zeros_like(x)], axis=0).astype(BF16), U32)


def _dot(a, b):
    return jnp.dot(a, b, preferred_element_type=F32)


def _lanes(i):
    return slice(i * LANES, (i + 1) * LANES)


def _make_kernel(D, F, SK, W):
    NJ = W // LANES
    ND = D // LANES
    cexp = DH ** -0.5 * LOG2E

    def kernel(x_hbm, k_hbm, v_hbm, wq_hbm, wo_hbm, w1_hbm, w3_hbm, w2_hbm, o_ref,
               xb, kb, vb, wq, wo, w1, w3, w2,
               gq_ref, gs_ref, gp_ref, gacc_ref, act_ref,
               qm_ref, om_ref, lhs_ref, pm_ref, ob_ref, *rest):
        pv_refs, (sem_k, sem_v, sem_w) = rest[:NV], rest[NV:]

        def k_copy(j):
            return pltpu.make_async_copy(
                k_hbm.at[:, pl.ds(SK - W + j * LANES, LANES)], kb.at[j], sem_k.at[j])

        def v_copy(j):
            return pltpu.make_async_copy(
                v_hbm.at[:, pl.ds(SK - W + j * LANES, LANES)], vb.at[j], sem_v.at[j])

        def w2_copy(n):
            r = pl.ds(pl.multiple_of(n * QC, QC), QC)
            return pltpu.make_async_copy(w2_hbm.at[r], w2.at[r], sem_w.at[5 + n])

        def start(copy, j):
            @pl.when(j % 2 == 0)
            def _():
                copy(j).start(priority=0)

            @pl.when(j % 2 == 1)
            def _():
                copy(j).start(priority=PRIO)

        x_copy = pltpu.make_async_copy(x_hbm, xb, sem_w.at[0])
        wq_copy = pltpu.make_async_copy(wq_hbm, wq, sem_w.at[1])
        wo_copy = pltpu.make_async_copy(wo_hbm, wo, sem_w.at[2])
        w1_copy = pltpu.make_async_copy(w1_hbm, w1, sem_w.at[3])
        w3_copy = pltpu.make_async_copy(w3_hbm, w3, sem_w.at[4])

        x_copy.start()
        wq_copy.start()
        for j in range(AHEAD):
            k_copy(j).start(priority=PRIO * (j % 2))

        kbu = kb.bitcast(U32)
        vbu = vb.bitcast(U32)

        sub = lax.broadcasted_iota(jnp.int32, (8, PR), 0)
        lane = lax.broadcasted_iota(jnp.int32, (8, PR), 1)
        half = jnp.where(lane < DH, jnp.uint32(0x0000FFFF), jnp.uint32(0xFFFF0000))
        for ph in range(4):
            qm_ref[ph] = jnp.where(sub == ph, half, jnp.uint32(0))
        om_ref[...] = half

        def normed(x):
            return jnp.broadcast_to(_layernorm(x), (16, D)).astype(BF16)

        def attention1(x):
            row = lax.broadcasted_iota(jnp.int32, (HG, GR), 0)
            col = lax.broadcasted_iota(jnp.int32, (HG, GR), 1)
            diag = (col >= row * DH) & (col < (row + 1) * DH)
            h = normed(x)
            wq_copy.wait()

            @pl.loop(0, NG)
            def _(g):
                q = _dot(h, wq[:, pl.ds(pl.multiple_of(g * GR, GR), GR)])[0:HG]
                gq_ref[g] = _pack(jnp.where(diag, q, 0.0))

            def rows(g):
                return pl.ds(pl.multiple_of(g * (GR // 2), GR // 2), GR // 2)

            @pl.loop(0, NJ)
            def _(j):
                k_copy(j).wait()

                @pl.when(j + AHEAD < NJ)
                def _():
                    start(k_copy, j + AHEAD)

                @pl.when(j + AHEAD >= NJ)
                def _():
                    start(v_copy, j + AHEAD - NJ)

                @pl.loop(0, NG)
                def _(g):
                    gs_ref[g, j] = _dot(_bf(gq_ref[g]), _bf(kbu[j, rows(g), :]))[0:HG]

            @pl.loop(0, NG)
            def _(g):
                s = gs_ref[g]
                m = jnp.max(jnp.max(s, axis=0), axis=-1, keepdims=True)
                e = jnp.exp2((s - m[None]) * cexp)
                l = jnp.sum(jnp.sum(e, axis=0), axis=-1, keepdims=True)
                p = e * (1.0 / l)[None]
                gp_ref[g] = pltpu.bitcast(
                    jnp.concatenate([p, jnp.zeros_like(p)], axis=1).astype(BF16), U32)
                gacc_ref[g] = jnp.zeros((HG, GR), F32)

            def pv(j, carry):
                v_copy(j).wait()

                @pl.when(j + AHEAD < NJ)
                def _():
                    start(v_copy, j + AHEAD)

                @pl.when(j + AHEAD == NJ)
                def _():
                    wo_copy.start()
                    w1_copy.start()
                    w3_copy.start()
                    for n in range(F // QC):
                        w2_copy(n).start()

                for g in range(NG):
                    vt = _bf(vbu[j, g * GR // 2:(g + 1) * GR // 2, :])
                    o = lax.dot_general(_bf(gp_ref[g, j]), vt, (((1,), (1,)), ((), ())),
                                        preferred_element_type=F32)
                    gacc_ref[g] += o[0:HG]
                    for t in range(GR // LANES):
                        r0 = g * GR + t * LANES
                        if r0 >= NV * PR:
                            vbu[j, r0 // 2:(r0 + LANES) // 2, :] = pltpu.bitcast(
                                vt[_lanes(t)].T, U32)
                return carry + j // NJ

            zero = lax.fori_loop(0, NJ, pv, jnp.int32(0))

            @pl.loop(0, NG)
            def _(g):
                gq_ref[g] = _pack(jnp.where(diag, gacc_ref[g], 0.0))

            wo_copy.wait()

            def project(g, y):
                r = pl.ds(pl.multiple_of(g * GR, GR), GR)
                return y + _dot(_bf(gq_ref[g]), wo[r, :])[0:HG]

            y = lax.fori_loop(0, NG, project, jnp.zeros((HG, D), F32))
            return jnp.sum(y, axis=0, keepdims=True), zero

        def ffn1(x):
            h = normed(x)
            w1_copy.wait()
            w3_copy.wait()

            @pl.loop(0, F // QC)
            def _(n):
                cols = pl.ds(pl.multiple_of(n * QC, QC), QC)
                gate = _dot(h, w1[:, cols])
                up = _dot(h, w3[:, cols])
                act_ref[:, cols] = pltpu.bitcast(
                    (gate * jax.nn.sigmoid(gate) * up).astype(BF16), U32)

            def down(n, y):
                w2_copy(n).wait()
                r = pl.ds(pl.multiple_of(n * QC, QC), QC)
                return y + _dot(_bf(act_ref[:, r]), w2[r, :])[0:8]

            return lax.fori_loop(0, F // QC, down, jnp.zeros((8, D), F32))[0:1]

        def ffn2(x):
            h = normed(x)
            gate = _dot(h, w1[...])[0:8]
            up = _dot(h, w3[...])[0:8]
            a = _bf(_pack(gate * jax.nn.sigmoid(gate) * up))
            return _dot(a, w2[...])[0:1]

        def attention2(x, zero):
            h = normed(x)
            never = om_ref[:, 0:LANES] == jnp.uint32(0)
            out = [None] * ND
            st = {}

            def accumulate(c, y):
                out[c] = y if out[c] is None else out[c] + y

            def join(vals):
                us = [pltpu.bitcast(v, U32) for v in vals]
                while len(us) > 1:
                    us = [a | b for a, b in zip(us[0::2], us[1::2])] + us[len(us) // 2 * 2:]
                return us[0]

            def tie(u, after):
                if after is None:
                    return _bf(u)
                first = jnp.where(never, after, u[:, 0:LANES])
                return _bf(jnp.concatenate([first, u[:, LANES:]], axis=1))

            def q_chunk(n, after):
                q = _dot(tie(pltpu.bitcast(h, U32), after), wq[:, n * QC:(n + 1) * QC])[0:8]
                qu = _pack(q)
                for i in range(QC // LANES):
                    p, t = divmod(n * QC // LANES + i, PT)
                    for ph in range(4):
                        lhs_ref[p, :, _lanes(ph * PT + t)] = (
                            qu[:, _lanes(i)] & qm_ref[ph, :, _lanes(t)])
                return q[:, 0:LANES]

            def qk(p, jo, after):
                kt = jnp.concatenate(
                    [_bf(kbu[4 * jo + ph, p * PR // 2:(p + 1) * PR // 2, :]) for ph in range(4)],
                    axis=0)
                s = _dot(tie(lhs_ref[p], after), kt)[0:8]
                st.setdefault(("s", p), []).append(s)
                if jo == NJ // 4 - 1:
                    softmax(p)
                return s

            def softmax(p):
                ss = st["s", p]
                m = ss[0]
                for s in ss[1:]:
                    m = jnp.maximum(m, s)
                m = jnp.maximum(m, pltpu.roll(m, 4, 0))
                m = jnp.maximum(m, pltpu.roll(m, 2, 0))
                m = jnp.max(m, axis=-1, keepdims=True)
                l = None
                for jo, s in enumerate(ss):
                    e = jnp.exp2((s - m) * cexp)
                    l = e if l is None else l + e
                    if p < NV:
                        for sl in range(8):
                            pv_refs[p][(sl % 2) * NJ + 4 * jo + sl // 2] = jnp.broadcast_to(
                                e[sl:sl + 1], (8, LANES))
                    else:
                        eu = _pack(e)
                        for ph in range(4):
                            own = qm_ref[ph, :, 0:LANES] != jnp.uint32(0)
                            pm_ref[p - NV, :, _lanes(4 * jo + ph)] = jnp.where(
                                own, eu, jnp.uint32(0))
                l = l + pltpu.roll(l, 4, 0)
                l = l + pltpu.roll(l, 2, 0)
                st["inv", p] = 1.0 / jnp.sum(l, axis=-1, keepdims=True)

            def mxu_pv(p, t, part, after):
                j0, j1 = part * NJ // PVS, (part + 1) * NJ // PVS
                r0 = (p * PT + t) * (LANES // 2)
                vt = jnp.concatenate(
                    [_bf(vbu[j, r0:r0 + LANES // 2, :]) for j in range(j0, j1)], axis=0)
                o = _dot(tie(pm_ref[p - NV, :, j0 * LANES:j1 * LANES], after), vt)[0:8]
                if part:
                    o = o + st["o"]
                st["o"] = o
                if part == PVS - 1:
                    ob_ref[:, _lanes((p - NV) * PT + t)] = (
                        _pack(o * st["inv", p]) & om_ref[:, _lanes(t)])
                return o

            def mxu_wo(c, after):
                y = _dot(tie(ob_ref[...], after), wo[NV * PR:, _lanes(c)])[0:8]
                st["y", c] = y
                return y

            def vpu_wo():
                if "os" not in st:
                    return
                r0, os_ = st.pop("os")
                for c in range(ND):
                    wf = wo[r0:r0 + 16 * IB, _lanes(c)].astype(F32)
                    y = None
                    for a in range(2 * IB):
                        t = wf[8 * a:8 * a + 8] * os_[a]
                        y = t if y is None else y + t
                    accumulate(c, y)

            def vpu_pv(p, hd, blk, after):
                r0 = p * PR + hd * DH + blk * 16 * IB
                base = hd * NJ + (zero * (blk + 1) if NOCSE else 0)
                accs = [None] * (2 * IB)
                for j in range(NJ):
                    if j == WO_AT:
                        vpu_wo()
                    pj = pv_refs[p][base + j]
                    if j == DM_AT:
                        pj = jnp.where(never, after, pj)
                    vf = vb[j, r0:r0 + 16 * IB, :].astype(F32)
                    for a in range(2 * IB):
                        t = vf[8 * a:8 * a + 8] * pj
                        accs[a] = t if accs[a] is None else accs[a] + t
                if blk == 0:
                    st["scale"] = jnp.broadcast_to(st["inv", p][hd:hd + 1], (8, 1))
                st["os"] = (r0, [jnp.sum(a, axis=-1, keepdims=True) * st["scale"] for a in accs])
                return accs + [y for y in out if y is not None]

            mxu, nq = [], 0
            pv_tasks = lambda p: [(NJ // PVS, mxu_pv, (p, t, part))
                                  for t in range(PT) for part in range(PVS)]
            for p in range(NP):
                while nq * QC < (min(p + Q_AHEAD, NP) if p else 1) * PR:
                    mxu.append((ND * QC // LANES, q_chunk, (nq,)))
                    nq += 1
                mxu += [(4 * PT, qk, (p, jo)) for jo in range(NJ // 4)]
                if p > NV:
                    mxu += pv_tasks(p - 1)
            mxu += pv_tasks(NP - 1)
            mxu += [(PT * (NP - NV), mxu_wo, (c,)) for c in range(ND)]
            vpu = [(p, hd, blk) for p in range(NV) for hd in range(2)
                   for blk in range(DH // (16 * IB))]

            start, t, ready = [], 0, {}
            for tiles, fn, args in mxu:
                start.append(t)
                t += MXU_TILE * tiles // 10
                if fn is qk:
                    ready[args[0]] = t + SOFTMAX_LAT
            start.append(t)
            done, blocks, nxt, tv = [], [], 0, 0

            def issue(i):
                prev = [k for k, (end, _) in enumerate(blocks) if end + VPU_LAT <= start[i]]
                after = None
                if prev and prev[-1] >= st.get("tied", -1) + TIE_EVERY:
                    st["tied"] = prev[-1]
                    after = join(blocks[prev[-1]][1])
                done.append(mxu[i][1](*mxu[i][2], after))

            for p, hd, blk in vpu:
                tv = max(tv, ready[p])
                while nxt < len(mxu) and start[nxt] <= tv:
                    issue(nxt)
                    nxt += 1
                last = max(i for i in range(nxt) if start[i + 1] + MXU_LAT <= tv)
                tv += VPU_BLOCK
                blocks.append((tv, vpu_pv(p, hd, blk, done[last])))
            vpu_wo()
            for i in range(nxt, len(mxu)):
                issue(i)
            return jnp.concatenate(
                [jnp.sum(out[c] + st["y", c], axis=0, keepdims=True) for c in range(ND)], axis=1)

        x_copy.wait()
        x = xb[...].astype(F32)
        y, zero = attention1(x)
        x = _rnd(x + _rnd(y))
        x = _rnd(x + _rnd(ffn1(x)))
        x = _rnd(x + _rnd(attention2(x, zero)))
        x = _rnd(x + _rnd(ffn2(x)))
        o_ref[...] = x.astype(o_ref.dtype)

    return kernel


@jax.jit
def pallas_interleave_layers__sliding_block_cached__glu_gated_swiglu__decode_kernel(
    A_x: jax.Array,
    A_k_cache: jax.Array,
    A_v_cache: jax.Array,
    A_wq: jax.Array,
    A_wo: jax.Array,
    B_x: jax.Array,
    B_w1: jax.Array,
    B_w3: jax.Array,
    B_w2: jax.Array,
):
    del B_x
    D = A_x.shape[-1]
    F = B_w1.shape[-1]
    SK = A_k_cache.shape[2]
    W = min(4096, max(256, SK // 4))
    NJ = W // LANES
    ND = D // LANES

    k_t = jnp.swapaxes(A_k_cache[0], 1, 2).reshape(R, SK)
    v_t = jnp.swapaxes(A_v_cache[0], 1, 2).reshape(R, SK)

    hbm = pl.BlockSpec(memory_space=pl.ANY)
    out = pl.pallas_call(
        _make_kernel(D, F, SK, W),
        out_shape=jax.ShapeDtypeStruct((1, D), A_x.dtype),
        in_specs=[hbm] * 8,
        out_specs=pl.BlockSpec(memory_space=pltpu.VMEM),
        scratch_shapes=[
            pltpu.VMEM((1, D), BF16),
            pltpu.VMEM((NJ, R, LANES), BF16),
            pltpu.VMEM((NJ, R, LANES), BF16),
            pltpu.VMEM((D, R), BF16),
            pltpu.VMEM((R, D), BF16),
            pltpu.VMEM((D, F), BF16),
            pltpu.VMEM((D, F), BF16),
            pltpu.VMEM((F, D), BF16),
            pltpu.VMEM((NG, HG, GR), U32),
            pltpu.VMEM((NG, NJ, HG, LANES), F32),
            pltpu.VMEM((NG, NJ, HG, LANES), U32),
            pltpu.VMEM((NG, HG, GR), F32),
            pltpu.VMEM((8, F), U32),
            pltpu.VMEM((4, 8, PR), U32),
            pltpu.VMEM((8, PR), U32),
            pltpu.VMEM((NP, 8, 4 * PR), U32),
            pltpu.VMEM((NP - NV, 8, W), U32),
            pltpu.VMEM((8, (NP - NV) * PR), U32),
            *[pltpu.VMEM((2 * NJ, 8, LANES), F32)] * NV,
            pltpu.SemaphoreType.DMA((NJ,)),
            pltpu.SemaphoreType.DMA((NJ,)),
            pltpu.SemaphoreType.DMA((5 + F // QC,)),
        ],
        compiler_params=pltpu.CompilerParams(
            vmem_limit_bytes=127 * 1024 * 1024,
            disable_semaphore_checks=True,
            disable_bounds_checks=True,
        ),
    )(A_x.reshape(1, D), k_t, v_t, A_wq, A_wo, B_w1, B_w3, B_w2)
    return out.reshape(A_x.shape)
```

```python
import jax
import jax.numpy as jnp
from jax import lax
import jax.experimental.pallas as pl
import jax.experimental.pallas.tpu as pltpu

BF16 = jnp.bfloat16
F32 = jnp.float32
U32 = jnp.uint32

HQ, DH = 32, 192
R = HQ * DH
LANES = 128
HG = 8
NG = HQ // HG
GR = HG * DH
NP = HQ // 2
PR = 2 * DH
PT = PR // LANES
EPS = 1e-5
LOG2E = 1.4426950408889634

PRIO = 0
AHEAD = 4
QC = 512
NV = 11
IB = 2
MT = 4
DELAY = 0
JS = 8
DM = 8
LEAD = 0
Q_AHEAD = 2
SOFTMAX_LAT = 400
MXU_TILE = 85
VPU_BLOCK = 133
VPU_LAT = 250
TIE_EVERY = 1
WO_AT = 20
DM_AT = 7
NOCSE = 1


def _layernorm(x):
    m = jnp.mean(x, axis=-1, keepdims=True)
    c = x - m
    v = jnp.mean(c * c, axis=-1, keepdims=True)
    return c / jnp.sqrt(v + EPS)


def _rnd(x):
    return x.astype(BF16).astype(F32)


def _bf(u):
    return pltpu.bitcast(u, BF16)


def _pack(x):
    return pltpu.bitcast(jnp.concatenate([x, jnp.zeros_like(x)], axis=0).astype(BF16), U32)


def _dot(a, b):
    return jnp.dot(a, b, preferred_element_type=F32)


def _lanes(i):
    return slice(i * LANES, (i + 1) * LANES)


def _make_kernel(D, F, SK, W):
    NJ = W // LANES
    ND = D // LANES
    cexp = DH ** -0.5 * LOG2E

    def kernel(x_hbm, k_hbm, v_hbm, wq_hbm, wo_hbm, w1_hbm, w3_hbm, w2_hbm, o_ref,
               xb, kb, vb, wq, wo, w1, w3, w2,
               gq_ref, gs_ref, gp_ref, gacc_ref, act_ref,
               qm_ref, om_ref, lhs_ref, pm_ref, ob_ref, *rest):
        pv_refs, (sem_k, sem_v, sem_w) = rest[:NV], rest[NV:]

        def k_copy(j):
            return pltpu.make_async_copy(
                k_hbm.at[:, pl.ds(SK - W + j * LANES, LANES)], kb.at[j], sem_k.at[j])

        def v_copy(j):
            return pltpu.make_async_copy(
                v_hbm.at[:, pl.ds(SK - W + j * LANES, LANES)], vb.at[j], sem_v.at[j])

        def w2_copy(n):
            r = pl.ds(pl.multiple_of(n * QC, QC), QC)
            return pltpu.make_async_copy(w2_hbm.at[r], w2.at[r], sem_w.at[5 + n])

        def start(copy, j):
            @pl.when(j % 2 == 0)
            def _():
                copy(j).start(priority=0)

            @pl.when(j % 2 == 1)
            def _():
                copy(j).start(priority=PRIO)

        x_copy = pltpu.make_async_copy(x_hbm, xb, sem_w.at[0])
        wq_copy = pltpu.make_async_copy(wq_hbm, wq, sem_w.at[1])
        wo_copy = pltpu.make_async_copy(wo_hbm, wo, sem_w.at[2])
        w1_copy = pltpu.make_async_copy(w1_hbm, w1, sem_w.at[3])
        w3_copy = pltpu.make_async_copy(w3_hbm, w3, sem_w.at[4])

        x_copy.start()
        wq_copy.start()
        for j in range(AHEAD):
            k_copy(j).start(priority=PRIO * (j % 2))

        kbu = kb.bitcast(U32)
        vbu = vb.bitcast(U32)

        sub = lax.broadcasted_iota(jnp.int32, (8, PR), 0)
        lane = lax.broadcasted_iota(jnp.int32, (8, PR), 1)
        half = jnp.where(lane < DH, jnp.uint32(0x0000FFFF), jnp.uint32(0xFFFF0000))
        for ph in range(4):
            qm_ref[ph] = jnp.where(sub == ph, half, jnp.uint32(0))
        om_ref[...] = half

        def normed(x):
            return jnp.broadcast_to(_layernorm(x), (16, D)).astype(BF16)

        def attention1(x):
            row = lax.broadcasted_iota(jnp.int32, (HG, GR), 0)
            col = lax.broadcasted_iota(jnp.int32, (HG, GR), 1)
            diag = (col >= row * DH) & (col < (row + 1) * DH)
            h = normed(x)
            wq_copy.wait()

            @pl.loop(0, NG)
            def _(g):
                q = _dot(h, wq[:, pl.ds(pl.multiple_of(g * GR, GR), GR)])[0:HG]
                gq_ref[g] = _pack(jnp.where(diag, q, 0.0))

            def rows(g):
                return pl.ds(pl.multiple_of(g * (GR // 2), GR // 2), GR // 2)

            @pl.loop(0, NJ)
            def _(j):
                k_copy(j).wait()

                @pl.when(j + AHEAD < NJ)
                def _():
                    start(k_copy, j + AHEAD)

                @pl.when(j + AHEAD >= NJ)
                def _():
                    start(v_copy, j + AHEAD - NJ)

                @pl.loop(0, NG)
                def _(g):
                    gs_ref[g, j] = _dot(_bf(gq_ref[g]), _bf(kbu[j, rows(g), :]))[0:HG]

            @pl.loop(0, NG)
            def _(g):
                s = gs_ref[g]
                m = jnp.max(jnp.max(s, axis=0), axis=-1, keepdims=True)
                e = jnp.exp2((s - m[None]) * cexp)
                l = jnp.sum(jnp.sum(e, axis=0), axis=-1, keepdims=True)
                p = e * (1.0 / l)[None]
                gp_ref[g] = pltpu.bitcast(
                    jnp.concatenate([p, jnp.zeros_like(p)], axis=1).astype(BF16), U32)
                gacc_ref[g] = jnp.zeros((HG, GR), F32)

            def pv(j, carry):
                v_copy(j).wait()

                @pl.when(j + AHEAD < NJ)
                def _():
                    start(v_copy, j + AHEAD)

                @pl.when(j + AHEAD == NJ)
                def _():
                    wo_copy.start()
                    w1_copy.start()
                    w3_copy.start()
                    for n in range(F // QC):
                        w2_copy(n).start()

                for g in range(NG):
                    vt = _bf(vbu[j, g * GR // 2:(g + 1) * GR // 2, :])
                    o = lax.dot_general(_bf(gp_ref[g, j]), vt, (((1,), (1,)), ((), ())),
                                        preferred_element_type=F32)
                    gacc_ref[g] += o[0:HG]
                    for t in range(GR // LANES):
                        r0 = g * GR + t * LANES
                        if r0 >= NV * PR:
                            vbu[j, r0 // 2:(r0 + LANES) // 2, :] = pltpu.bitcast(
                                vt[_lanes(t)].T, U32)
                return carry + j // NJ

            zero = lax.fori_loop(0, NJ, pv, jnp.int32(0))

            @pl.loop(0, NG)
            def _(g):
                gq_ref[g] = _pack(jnp.where(diag, gacc_ref[g], 0.0))

            wo_copy.wait()

            def project(g, y):
                r = pl.ds(pl.multiple_of(g * GR, GR), GR)
                return y + _dot(_bf(gq_ref[g]), wo[r, :])[0:HG]

            y = lax.fori_loop(0, NG, project, jnp.zeros((HG, D), F32))
            return jnp.sum(y, axis=0, keepdims=True), zero

        def ffn1(x):
            h = normed(x)
            w1_copy.wait()
            w3_copy.wait()

            @pl.loop(0, F // QC)
            def _(n):
                cols = pl.ds(pl.multiple_of(n * QC, QC), QC)
                gate = _dot(h, w1[:, cols])
                up = _dot(h, w3[:, cols])
                act_ref[:, cols] = pltpu.bitcast(
                    (gate * jax.nn.sigmoid(gate) * up).astype(BF16), U32)

            def down(n, y):
                w2_copy(n).wait()
                r = pl.ds(pl.multiple_of(n * QC, QC), QC)
                return y + _dot(_bf(act_ref[:, r]), w2[r, :])[0:8]

            return lax.fori_loop(0, F // QC, down, jnp.zeros((8, D), F32))[0:1]

        def ffn2(x):
            h = normed(x)
            gate = _dot(h, w1[...])[0:8]
            up = _dot(h, w3[...])[0:8]
            a = _bf(_pack(gate * jax.nn.sigmoid(gate) * up))
            return _dot(a, w2[...])[0:1]

        def attention2(x, zero):
            h = normed(x)
            never = om_ref[:, 0:LANES] == jnp.uint32(0)
            out = [None] * ND
            st = {}

            def accumulate(c, y):
                out[c] = y if out[c] is None else out[c] + y

            def join(vals):
                us = [pltpu.bitcast(v, U32) for v in vals]
                while len(us) > 1:
                    us = [a | b for a, b in zip(us[0::2], us[1::2])] + us[len(us) // 2 * 2:]
                return us[0]

            def tie(u, after):
                if after is None:
                    return _bf(u)
                first = jnp.where(never, after, u[:, 0:LANES])
                if u.shape[1] == LANES:
                    return _bf(first)
                return _bf(jnp.concatenate([first, u[:, LANES:]], axis=1))

            def chain(lhs, rhs, n):
                acc, pending = None, []
                for k in range(0, n, MT):
                    m = min(MT, n - k)
                    after = yield m
                    pending.append(_dot(tie(lhs(k, m), after), rhs(k, m))[0:8])
                    if len(pending) > DELAY:
                        y = pending.pop(0)
                        acc = y if acc is None else acc + y
                        st["done"] = acc
                for y in pending:
                    acc = y if acc is None else acc + y
                return acc

            def q_chunk(n):
                hu = pltpu.bitcast(h, U32)
                q = None
                for k in range(ND):
                    after = yield QC // LANES
                    hk = hu[:, _lanes(k)]
                    if after is not None:
                        hk = jnp.where(never, after, hk)
                    y = _dot(_bf(hk), wq[_lanes(k), n * QC:(n + 1) * QC])[0:8]
                    q = y if q is None else q + y
                qu = _pack(q)
                for i in range(QC // LANES):
                    p, t = divmod(n * QC // LANES + i, PT)
                    for ph in range(4):
                        lhs_ref[p, :, _lanes(ph * PT + t)] = (
                            qu[:, _lanes(i)] & qm_ref[ph, :, _lanes(t)])
                st["done"] = q[:, 0:LANES]

            def tile(ref, j, t):
                return _bf(ref[j, t * LANES // 2:(t + 1) * LANES // 2, :])

            def qk(p, jo):
                s = yield from chain(
                    lambda k, m: lhs_ref[p, :, k * LANES:(k + m) * LANES],
                    lambda k, m: jnp.concatenate(
                        [tile(kbu, 4 * jo + i // PT, p * PT + i % PT) for i in range(k, k + m)],
                        axis=0),
                    4 * PT)
                st["done"] = s
                st.setdefault(("s", p), []).append(s)
                if jo == NJ // 4 - 1:
                    softmax(p)
                    st["ready", p] = st["tm"] + SOFTMAX_LAT

            def softmax(p):
                ss = st["s", p]
                m = ss[0]
                for s in ss[1:]:
                    m = jnp.maximum(m, s)
                m = jnp.maximum(m, pltpu.roll(m, 4, 0))
                m = jnp.maximum(m, pltpu.roll(m, 2, 0))
                m = jnp.max(m, axis=-1, keepdims=True)
                l = None
                for jo, s in enumerate(ss):
                    e = jnp.exp2((s - m) * cexp)
                    l = e if l is None else l + e
                    if p < NV:
                        for sl in range(8):
                            pv_refs[p][(sl % 2) * NJ + 4 * jo + sl // 2] = jnp.broadcast_to(
                                e[sl:sl + 1], (8, LANES))
                    else:
                        eu = _pack(e)
                        for ph in range(4):
                            own = qm_ref[ph, :, 0:LANES] != jnp.uint32(0)
                            pm_ref[p - NV, :, _lanes(4 * jo + ph)] = jnp.where(
                                own, eu, jnp.uint32(0))
                l = l + pltpu.roll(l, 4, 0)
                l = l + pltpu.roll(l, 2, 0)
                st["inv", p] = 1.0 / jnp.sum(l, axis=-1, keepdims=True)

            def mxu_pv(p, t):
                o = yield from chain(
                    lambda k, m: pm_ref[p - NV, :, k * LANES:(k + m) * LANES],
                    lambda k, m: jnp.concatenate(
                        [tile(vbu, i, p * PT + t) for i in range(k, k + m)], axis=0),
                    NJ)
                ob_ref[:, _lanes((p - NV) * PT + t)] = (
                    _pack(o * st["inv", p]) & om_ref[:, _lanes(t)])

            def mxu_wo(c):
                st["y", c] = yield from chain(
                    lambda k, m: ob_ref[:, k * LANES:(k + m) * LANES],
                    lambda k, m: wo[NV * PR + k * LANES:NV * PR + (k + m) * LANES, _lanes(c)],
                    (NP - NV) * PT)

            def vpu_wo():
                if "os" not in st:
                    return
                r0, os_ = st.pop("os")
                for c in range(ND):
                    wf = wo[r0:r0 + 16 * IB, _lanes(c)].astype(F32)
                    y = None
                    for a in range(2 * IB):
                        t = wf[8 * a:8 * a + 8] * os_[a]
                        y = t if y is None else y + t
                    accumulate(c, y)

            def vpu_pv(p, hd, blk):
                r0 = p * PR + hd * DH + blk * 16 * IB
                base = hd * NJ + (zero * (blk + 1) if NOCSE else 0)
                accs = [None] * (2 * IB)
                for j in range(NJ):
                    if j % JS == 0:
                        yield JS
                    if j == WO_AT:
                        vpu_wo()
                    pj = pv_refs[p][base + j]
                    if j % DM == DM_AT:
                        pj = jnp.where(never, st["done"], pj)
                    vf = vb[j, r0:r0 + 16 * IB, :].astype(F32)
                    for a in range(2 * IB):
                        t = vf[8 * a:8 * a + 8] * pj
                        accs[a] = t if accs[a] is None else accs[a] + t
                if blk == 0:
                    st["scale"] = jnp.broadcast_to(st["inv", p][hd:hd + 1], (8, 1))
                st["os"] = (r0, [jnp.sum(a, axis=-1, keepdims=True) * st["scale"] for a in accs])
                blocks.append((st["tv"], accs + [y for y in out if y is not None]))

            def mxu_stream():
                nq = 0
                for p in range(NP):
                    while nq * QC < (min(p + Q_AHEAD, NP) if p else 1) * PR:
                        yield from q_chunk(nq)
                        nq += 1
                    for jo in range(NJ // 4):
                        yield from qk(p, jo)
                    if p > NV:
                        for t in range(PT):
                            yield from mxu_pv(p - 1, t)
                for t in range(PT):
                    yield from mxu_pv(NP - 1, t)
                for c in range(ND):
                    yield from mxu_wo(c)

            blocks = []
            st["tm"] = st["tv"] = 0
            mxu = mxu_stream()
            st["tiles"] = next(mxu)

            def mxu_step():
                prev = [k for k, (end, _) in enumerate(blocks) if end + VPU_LAT <= st["tm"]]
                after = None
                if prev and prev[-1] >= st.get("tied", -1) + TIE_EVERY:
                    st["tied"] = prev[-1]
                    after = join(blocks[prev[-1]][1])
                st["tm"] += MXU_TILE * st["tiles"] / 10
                try:
                    st["tiles"] = mxu.send(after)
                except StopIteration:
                    st["tiles"] = None

            for p in range(NV):
                while ("ready", p) not in st:
                    mxu_step()
                st["tv"] = max(st["tv"], st["ready", p])
                for hd in range(2):
                    for blk in range(DH // (16 * IB)):
                        for steps in vpu_pv(p, hd, blk):
                            while st["tiles"] and st["tm"] <= st["tv"] + LEAD:
                                mxu_step()
                            st["tv"] += VPU_BLOCK * steps / NJ
            vpu_wo()
            while st["tiles"]:
                mxu_step()
            return jnp.concatenate(
                [jnp.sum(out[c] + st["y", c], axis=0, keepdims=True) for c in range(ND)], axis=1)

        x_copy.wait()
        x = xb[...].astype(F32)
        y, zero = attention1(x)
        x = _rnd(x + _rnd(y))
        x = _rnd(x + _rnd(ffn1(x)))
        x = _rnd(x + _rnd(attention2(x, zero)))
        x = _rnd(x + _rnd(ffn2(x)))
        o_ref[...] = x.astype(o_ref.dtype)

    return kernel


@jax.jit
def pallas_interleave_layers__sliding_block_cached__glu_gated_swiglu__decode_kernel(
    A_x: jax.Array,
    A_k_cache: jax.Array,
    A_v_cache: jax.Array,
    A_wq: jax.Array,
    A_wo: jax.Array,
    B_x: jax.Array,
    B_w1: jax.Array,
    B_w3: jax.Array,
    B_w2: jax.Array,
):
    del B_x
    D = A_x.shape[-1]
    F = B_w1.shape[-1]
    SK = A_k_cache.shape[2]
    W = min(4096, max(256, SK // 4))
    NJ = W // LANES
    ND = D // LANES

    k_t = jnp.swapaxes(A_k_cache[0], 1, 2).reshape(R, SK)
    v_t = jnp.swapaxes(A_v_cache[0], 1, 2).reshape(R, SK)

    hbm = pl.BlockSpec(memory_space=pl.ANY)
    out = pl.pallas_call(
        _make_kernel(D, F, SK, W),
        out_shape=jax.ShapeDtypeStruct((1, D), A_x.dtype),
        in_specs=[hbm] * 8,
        out_specs=pl.BlockSpec(memory_space=pltpu.VMEM),
        scratch_shapes=[
            pltpu.VMEM((1, D), BF16),
            pltpu.VMEM((NJ, R, LANES), BF16),
            pltpu.VMEM((NJ, R, LANES), BF16),
            pltpu.VMEM((D, R), BF16),
            pltpu.VMEM((R, D), BF16),
            pltpu.VMEM((D, F), BF16),
            pltpu.VMEM((D, F), BF16),
            pltpu.VMEM((F, D), BF16),
            pltpu.VMEM((NG, HG, GR), U32),
            pltpu.VMEM((NG, NJ, HG, LANES), F32),
            pltpu.VMEM((NG, NJ, HG, LANES), U32),
            pltpu.VMEM((NG, HG, GR), F32),
            pltpu.VMEM((8, F), U32),
            pltpu.VMEM((4, 8, PR), U32),
            pltpu.VMEM((8, PR), U32),
            pltpu.VMEM((NP, 8, 4 * PR), U32),
            pltpu.VMEM((NP - NV, 8, W), U32),
            pltpu.VMEM((8, (NP - NV) * PR), U32),
            *[pltpu.VMEM((2 * NJ, 8, LANES), F32)] * NV,
            pltpu.SemaphoreType.DMA((NJ,)),
            pltpu.SemaphoreType.DMA((NJ,)),
            pltpu.SemaphoreType.DMA((5 + F // QC,)),
        ],
        compiler_params=pltpu.CompilerParams(
            vmem_limit_bytes=127 * 1024 * 1024,
            disable_semaphore_checks=True,
            disable_bounds_checks=True,
        ),
    )(A_x.reshape(1, D), k_t, v_t, A_wq, A_wo, B_w1, B_w3, B_w2)
    return out.reshape(A_x.shape)
```

```python
import jax
import jax.numpy as jnp
from jax import lax
import jax.experimental.pallas as pl
import jax.experimental.pallas.tpu as pltpu

BF16 = jnp.bfloat16
F32 = jnp.float32
U32 = jnp.uint32

HQ, DH = 32, 192
R = HQ * DH
LANES = 128
HG = 8
NG = HQ // HG
GR = HG * DH
NP = HQ // 2
PR = 2 * DH
PT = PR // LANES
EPS = 1e-5
LOG2E = 1.4426950408889634

PRIO = 1
AHEAD = 4
QC = 512
NV = 10
IB = 2
MT = 4
JS = 8
DM = 8
QPART = 20
NQV = 8
NFV = 2
COL_LAT = 200
Q_STEP = 36
Q_AHEAD = 2
SOFTMAX_LAT = 400
MXU_TILE = 85
VPU_BLOCK = 136
VPU_LAT = 250
TIE_EVERY = 2
WO_AT = 20
DM_AT = 5


def _layernorm(x):
    m = jnp.mean(x, axis=-1, keepdims=True)
    c = x - m
    v = jnp.mean(c * c, axis=-1, keepdims=True)
    return c / jnp.sqrt(v + EPS)


def _rnd(x):
    return x.astype(BF16).astype(F32)


def _bf(u):
    return pltpu.bitcast(u, BF16)


def _pack(x):
    return pltpu.bitcast(jnp.concatenate([x, jnp.zeros_like(x)], axis=0).astype(BF16), U32)


def _dot(a, b):
    return jnp.dot(a, b, preferred_element_type=F32)


def _lanes(i):
    return slice(i * LANES, (i + 1) * LANES)


class _Streams:
    def __init__(self, never, mxu):
        self.never = never
        self.mxu = mxu
        self.tm, self.tv = 0, COL_LAT
        self.mxu_result = None
        self.vpu_results = []
        self.tied = -1
        self.tiles = next(mxu)

    def after_mxu(self, i, v):
        if i % DM == DM_AT and self.mxu_result is not None:
            return jnp.where(self.never, self.mxu_result, v)
        return v

    def after_vpu(self, u):
        prev = [k for k, (t, _) in enumerate(self.vpu_results) if t + VPU_LAT <= self.tm]
        if not prev or prev[-1] < self.tied + TIE_EVERY:
            return _bf(u)
        self.tied = prev[-1]
        us = [pltpu.bitcast(v, U32) for v in self.vpu_results[self.tied][1]]
        while len(us) > 1:
            us = [a | b for a, b in zip(us[0::2], us[1::2])] + us[len(us) // 2 * 2:]
        first = jnp.where(self.never, us[0], u[:, 0:LANES])
        if u.shape[1] == LANES:
            return _bf(first)
        return _bf(jnp.concatenate([first, u[:, LANES:]], axis=1))

    def vpu_done(self, values):
        self.vpu_results.append((self.tv, values))

    def mxu_step(self):
        tiles, self.tiles = self.tiles, next(self.mxu, None)
        self.tm += MXU_TILE * tiles / 10

    def vpu_run(self, task, cost):
        for steps in task:
            while self.tiles and self.tm <= self.tv:
                self.mxu_step()
            self.tv += cost * steps

    def finish(self):
        while self.tiles:
            self.mxu_step()

    def chain(self, lhs, rhs, n, step):
        acc = None
        for k in range(0, n, step):
            m = min(step, n - k)
            yield MT * m / step
            y = _dot(self.after_vpu(lhs(k, m)), rhs(k, m))[0:8]
            acc = y if acc is None else acc + y
            self.mxu_result = acc[:, 0:LANES]
        return acc


def _make_kernel(D, F, SK, W):
    NJ = W // LANES
    ND = D // LANES
    cexp = DH ** -0.5 * LOG2E

    def kernel(x_hbm, k_hbm, v_hbm, wq_hbm, wo_hbm, w1_hbm, w3_hbm, w2_hbm, o_ref,
               xb, kb, vb, wq, wo, w1, w3, w2,
               gq_ref, gs_ref, gp_ref, gacc_ref, act_ref,
               qm_ref, om_ref, hc_ref, lhs_ref, pm_ref, ob_ref, *rest):
        pv_refs, sems = rest[:NV], rest[NV]

        def k_copy(j):
            return pltpu.make_async_copy(
                k_hbm.at[:, pl.ds(SK - W + j * LANES, LANES)], kb.at[j], sems.at[j % AHEAD])

        def v_copy(j):
            return pltpu.make_async_copy(
                v_hbm.at[:, pl.ds(SK - W + j * LANES, LANES)], vb.at[j], sems.at[j % AHEAD])

        def rows_copy(src, dst, r0, n, sem):
            return pltpu.make_async_copy(
                src.at[pl.ds(r0, n)], dst.at[pl.ds(r0, n)], sems.at[sem])

        def start(copy, j, q):
            copy(j).start(priority=PRIO * q)

        def start_both(copies):
            for q, c in enumerate(copies):
                c.start(priority=PRIO * q)

        def wait(copies):
            for c in copies:
                c.wait()

        x_copy = pltpu.make_async_copy(x_hbm, xb, sems.at[AHEAD + 2])
        wq_copy = [rows_copy(wq_hbm, wq, q * D // 2, D // 2, AHEAD + q) for q in range(2)]
        wo_copy = [rows_copy(wo_hbm, wo, q * R // 2, R // 2, AHEAD + q) for q in range(2)]
        w13_copy = [pltpu.make_async_copy(w1_hbm, w1, sems.at[0]),
                    pltpu.make_async_copy(w3_hbm, w3, sems.at[1])]
        w2_copy = [[rows_copy(w2_hbm, w2, n * QC + q * QC // 2, QC // 2, sem + q)
                    for q in range(2)] for n, sem in enumerate((2, AHEAD, 0))]

        x_copy.start()
        start_both(wq_copy)
        for j in range(AHEAD):
            start(k_copy, j, j % 2)

        kbu = kb.bitcast(U32)
        vbu = vb.bitcast(U32)

        sub = lax.broadcasted_iota(jnp.int32, (8, PR), 0)
        lane = lax.broadcasted_iota(jnp.int32, (8, PR), 1)
        half = jnp.where(lane < DH, jnp.uint32(0x0000FFFF), jnp.uint32(0xFFFF0000))
        for ph in range(4):
            qm_ref[ph] = jnp.where(sub == ph, half, jnp.uint32(0))
        om_ref[...] = half

        def normed(x):
            return jnp.broadcast_to(_layernorm(x), (16, D)).astype(BF16)

        def normed2(x):
            h = normed(x)
            hf = h[0:8].astype(F32)
            for k in range(ND):
                hc_ref[_lanes(k), :] = jnp.concatenate([hf[:, _lanes(k)]] * (LANES // 8), axis=0).T
            return pltpu.bitcast(h, U32)

        def mxu_project(sm, hu, slabs):
            return sm().chain(
                lambda k, m: hu[:, _lanes(k)],
                lambda k, m: jnp.concatenate(
                    [w[_lanes(k), c0:c0 + 2 * LANES] for w, c0 in slabs], axis=1),
                ND, 1)

        def vpu_project(sm, slabs):
            accs = [None] * (2 * len(slabs))
            for i in range(D // 8):
                if i % JS == 0:
                    yield JS
                hi = sm().after_mxu(i, hc_ref[8 * i:8 * i + 8, :])
                for n, (w, c0) in enumerate(slabs):
                    wf = w[8 * i:8 * i + 8, c0:c0 + 2 * LANES].astype(F32)
                    for u in range(2):
                        t = wf[:, _lanes(u)] * hi
                        accs[2 * n + u] = t if i == 0 else accs[2 * n + u] + t
                if i % QPART == QPART - 1:
                    sm().vpu_done(list(accs))
            for shift in (4, 2, 1):
                accs = [a + pltpu.roll(a, shift, 0) for a in accs]
            return jnp.concatenate(accs, axis=1)

        def attention1(x):
            row = lax.broadcasted_iota(jnp.int32, (HG, GR), 0)
            col = lax.broadcasted_iota(jnp.int32, (HG, GR), 1)
            diag = (col >= row * DH) & (col < (row + 1) * DH)
            h = normed(x)
            wait(wq_copy)

            @pl.loop(0, NG)
            def _(g):
                q = _dot(h, wq[:, pl.ds(pl.multiple_of(g * GR, GR), GR)])[0:HG]
                gq_ref[g] = _pack(jnp.where(diag, q, 0.0))

            def rows(g):
                return pl.ds(pl.multiple_of(g * (GR // 2), GR // 2), GR // 2)

            @pl.loop(0, NJ, step=2)
            def _(j0):
                k_copy(j0).wait()
                k_copy(j0 + 1).wait()

                @pl.when(j0 + AHEAD < NJ)
                def _():
                    for q in range(2):
                        start(k_copy, j0 + q + AHEAD, q)

                @pl.when(j0 + AHEAD >= NJ)
                def _():
                    for q in range(2):
                        start(v_copy, j0 + q + AHEAD - NJ, q)

                @pl.loop(0, 2 * NG)
                def _(i):
                    j, g = j0 + i // NG, i % NG
                    gs_ref[g, j] = _dot(_bf(gq_ref[g]), _bf(kbu[j, rows(g), :]))[0:HG]

            @pl.loop(0, NG)
            def _(g):
                s = gs_ref[g]
                m = jnp.max(jnp.max(s, axis=0), axis=-1, keepdims=True)
                e = jnp.exp2((s - m[None]) * cexp)
                l = jnp.sum(jnp.sum(e, axis=0), axis=-1, keepdims=True)
                p = e * (1.0 / l)[None]
                gp_ref[g] = pltpu.bitcast(
                    jnp.concatenate([p, jnp.zeros_like(p)], axis=1).astype(BF16), U32)
                gacc_ref[g] = jnp.zeros((HG, GR), F32)

            @pl.loop(0, NJ)
            def _(j):
                v_copy(j).wait()

                for q in range(2):
                    @pl.when((j + AHEAD < NJ) & (j % 2 == q))
                    def _():
                        start(v_copy, j + AHEAD, q)

                @pl.when(j + AHEAD == NJ + 1)
                def _():
                    start_both(wo_copy)

                for g in range(NG):
                    vt = _bf(vbu[j, g * GR // 2:(g + 1) * GR // 2, :])
                    o = lax.dot_general(_bf(gp_ref[g, j]), vt, (((1,), (1,)), ((), ())),
                                        preferred_element_type=F32)
                    gacc_ref[g] += o[0:HG]
                    for t in range(GR // LANES):
                        r0 = g * GR + t * LANES
                        if r0 >= NV * PR:
                            vbu[j, r0 // 2:(r0 + LANES) // 2, :] = pltpu.bitcast(
                                vt[_lanes(t)].T, U32)

            start_both(w13_copy)

            @pl.loop(0, NG)
            def _(g):
                gq_ref[g] = _pack(jnp.where(diag, gacc_ref[g], 0.0))

            wait(wo_copy)

            def project(g, y):
                r = pl.ds(pl.multiple_of(g * GR, GR), GR)
                return y + _dot(_bf(gq_ref[g]), wo[r, :])[0:HG]

            y = lax.fori_loop(0, NG, project, jnp.zeros((HG, D), F32))
            start_both(w2_copy[0])
            return jnp.sum(y, axis=0, keepdims=True)

        def ffn1(x):
            h = normed(x)
            wait(w13_copy)
            start_both(w2_copy[1])

            @pl.loop(0, F // QC)
            def _(n):
                cols = pl.ds(pl.multiple_of(n * QC, QC), QC)
                gate = _dot(h, w1[:, cols])
                up = _dot(h, w3[:, cols])
                act_ref[:, cols] = pltpu.bitcast(
                    (gate * jax.nn.sigmoid(gate) * up).astype(BF16), U32)

            start_both(w2_copy[2])
            y = 0.0
            for n in range(F // QC):
                wait(w2_copy[n])
                y = y + _dot(_bf(act_ref[:, n * QC:(n + 1) * QC]), w2[n * QC:(n + 1) * QC, :])[0:1]
            return y

        def ffn2(x):
            hu = normed2(x)
            sm = lambda: streams
            nm = F // (2 * LANES) - NFV
            out = []

            def gated(project, n):
                c0 = 2 * LANES * n
                y = yield from project([(w1, c0), (w3, c0)])
                gate, up = y[:, 0:2 * LANES], y[:, 2 * LANES:]
                act_ref[:, c0:c0 + 2 * LANES] = _pack(gate * jax.nn.sigmoid(gate) * up)

            def down(k0, k1):
                for c in range(ND):
                    out.append((yield from streams.chain(
                        lambda k, m: act_ref[:, (k0 + k) * LANES:(k0 + k + m) * LANES],
                        lambda k, m: w2[(k0 + k) * LANES:(k0 + k + m) * LANES, _lanes(c)],
                        k1 - k0, MT)))

            def mxu_stream():
                yield 0.1
                for n in range(nm):
                    yield from gated(lambda slabs: mxu_project(sm, hu, slabs), n)
                yield from down(0, 2 * nm)

            streams = _Streams(om_ref[:, 0:LANES] == jnp.uint32(0), mxu_stream())
            for n in range(nm, nm + NFV):
                streams.vpu_run(gated(lambda slabs: vpu_project(sm, slabs), n), Q_STEP / 10)
            streams.finish()
            for _ in down(2 * nm, F // LANES):
                pass
            return jnp.concatenate(
                [sum(out[c + ND::ND], out[c])[0:1] for c in range(ND)], axis=1)

        def attention2(x):
            hu = normed2(x)
            sm = lambda: streams
            out = [None] * ND
            st = {}

            def accumulate(c, y):
                out[c] = y if out[c] is None else out[c] + y

            def q_chunk(project, n):
                q = yield from project([(wq, n * QC), (wq, n * QC + QC // 2)])
                qu = _pack(q)
                for i in range(QC // LANES):
                    p, t = divmod(n * QC // LANES + i, PT)
                    for ph in range(4):
                        lhs_ref[p, :, _lanes(ph * PT + t)] = (
                            qu[:, _lanes(i)] & qm_ref[ph, :, _lanes(t)])

            def tile(ref, j, t):
                return _bf(ref[j, t * LANES // 2:(t + 1) * LANES // 2, :])

            def qk(p):
                ss = []
                for jo in range(NJ // 4):
                    ss.append((yield from streams.chain(
                        lambda k, m: lhs_ref[p, :, k * LANES:(k + m) * LANES],
                        lambda k, m: jnp.concatenate(
                            [tile(kbu, 4 * jo + i // PT, p * PT + i % PT)
                             for i in range(k, k + m)], axis=0),
                        4 * PT, MT)))
                softmax(p, ss)
                st["ready", p] = streams.tm + SOFTMAX_LAT

            def softmax(p, ss):
                m = ss[0]
                for s in ss[1:]:
                    m = jnp.maximum(m, s)
                m = jnp.maximum(m, pltpu.roll(m, 4, 0))
                m = jnp.maximum(m, pltpu.roll(m, 2, 0))
                m = jnp.max(m, axis=-1, keepdims=True)
                l = None
                for jo, s in enumerate(ss):
                    e = jnp.exp2((s - m) * cexp)
                    l = e if l is None else l + e
                    if p < NV:
                        for sl in range(8):
                            pv_refs[p][(sl % 2) * NJ + 4 * jo + sl // 2] = jnp.broadcast_to(
                                e[sl:sl + 1], (8, LANES))
                    else:
                        eu = _pack(e)
                        for ph in range(4):
                            own = qm_ref[ph, :, 0:LANES] != jnp.uint32(0)
                            pm_ref[p - NV, :, _lanes(4 * jo + ph)] = jnp.where(
                                own, eu, jnp.uint32(0))
                l = l + pltpu.roll(l, 4, 0)
                l = l + pltpu.roll(l, 2, 0)
                st["inv", p] = 1.0 / jnp.sum(l, axis=-1, keepdims=True)

            def mxu_pv(p, t):
                o = yield from streams.chain(
                    lambda k, m: pm_ref[p - NV, :, k * LANES:(k + m) * LANES],
                    lambda k, m: jnp.concatenate(
                        [tile(vbu, i, p * PT + t) for i in range(k, k + m)], axis=0),
                    NJ, MT)
                ob_ref[:, _lanes((p - NV) * PT + t)] = (
                    _pack(o * st["inv", p]) & om_ref[:, _lanes(t)])

            def mxu_wo(c):
                st["y", c] = yield from streams.chain(
                    lambda k, m: ob_ref[:, k * LANES:(k + m) * LANES],
                    lambda k, m: wo[NV * PR + k * LANES:NV * PR + (k + m) * LANES, _lanes(c)],
                    (NP - NV) * PT, MT)

            def vpu_wo():
                if "os" not in st:
                    return
                r0, os_ = st.pop("os")
                for c in range(ND):
                    wf = wo[r0:r0 + 16 * IB, _lanes(c)].astype(F32)
                    y = None
                    for a in range(2 * IB):
                        t = wf[8 * a:8 * a + 8] * os_[a]
                        y = t if y is None else y + t
                    accumulate(c, y)

            def vpu_pv(p, hd, blk):
                r0 = p * PR + hd * DH + blk * 16 * IB
                base = hd * NJ
                accs = [None] * (2 * IB)
                for j in range(NJ):
                    if j % JS == 0:
                        yield JS
                    if j == WO_AT:
                        vpu_wo()
                    pj = streams.after_mxu(j, pv_refs[p][base + j])
                    vf = vb[j, r0:r0 + 16 * IB, :].astype(F32)
                    for a in range(2 * IB):
                        t = vf[8 * a:8 * a + 8] * pj
                        accs[a] = t if accs[a] is None else accs[a] + t
                if blk == 0:
                    st["scale"] = jnp.broadcast_to(st["inv", p][hd:hd + 1], (8, 1))
                st["os"] = (r0, [jnp.sum(a, axis=-1, keepdims=True) * st["scale"] for a in accs])
                streams.vpu_done(accs + [y for y in out if y is not None])

            def mxu_stream():
                yield 0.1
                nq = 0
                for p in range(NP):
                    while nq < R // QC - NQV and nq * QC < (p + Q_AHEAD if p else 1) * PR:
                        yield from q_chunk(lambda slabs: mxu_project(sm, hu, slabs), nq)
                        nq += 1
                    yield from qk(p)
                    if p > NV:
                        for t in range(PT):
                            yield from mxu_pv(p - 1, t)
                for t in range(PT):
                    yield from mxu_pv(NP - 1, t)
                for c in range(ND):
                    yield from mxu_wo(c)

            streams = _Streams(om_ref[:, 0:LANES] == jnp.uint32(0), mxu_stream())
            for n in range(R // QC - NQV, R // QC):
                streams.vpu_run(q_chunk(lambda slabs: vpu_project(sm, slabs), n), Q_STEP / 10)
            for p in range(NV):
                while ("ready", p) not in st:
                    streams.mxu_step()
                streams.tv = max(streams.tv, st["ready", p])
                for hd in range(2):
                    for blk in range(DH // (16 * IB)):
                        streams.vpu_run(vpu_pv(p, hd, blk), VPU_BLOCK / NJ)
            vpu_wo()
            streams.finish()
            return jnp.concatenate(
                [jnp.sum(out[c] + st["y", c], axis=0, keepdims=True) for c in range(ND)], axis=1)

        x_copy.wait()
        x = xb[...].astype(F32)
        x = _rnd(x + _rnd(attention1(x)))
        x = _rnd(x + _rnd(ffn1(x)))
        x = _rnd(x + _rnd(attention2(x)))
        x = _rnd(x + _rnd(ffn2(x)))
        o_ref[...] = x.astype(o_ref.dtype)

    return kernel


@jax.jit
def pallas_interleave_layers__sliding_block_cached__glu_gated_swiglu__decode_kernel(
    A_x: jax.Array,
    A_k_cache: jax.Array,
    A_v_cache: jax.Array,
    A_wq: jax.Array,
    A_wo: jax.Array,
    B_x: jax.Array,
    B_w1: jax.Array,
    B_w3: jax.Array,
    B_w2: jax.Array,
):
    del B_x
    D = A_x.shape[-1]
    F = B_w1.shape[-1]
    SK = A_k_cache.shape[2]
    W = min(4096, max(256, SK // 4))
    NJ = W // LANES
    ND = D // LANES

    k_t = jnp.swapaxes(A_k_cache, 2, 3).reshape(R, SK)
    v_t = jnp.swapaxes(A_v_cache, 2, 3).reshape(R, SK)

    hbm = pl.BlockSpec(memory_space=pl.ANY)
    out = pl.pallas_call(
        _make_kernel(D, F, SK, W),
        out_shape=jax.ShapeDtypeStruct((1, D), A_x.dtype),
        in_specs=[hbm] * 8,
        out_specs=pl.BlockSpec(memory_space=pltpu.VMEM),
        scratch_shapes=[
            pltpu.VMEM((1, D), BF16),
            pltpu.VMEM((NJ, R, LANES), BF16),
            pltpu.VMEM((NJ, R, LANES), BF16),
            pltpu.VMEM((D, R), BF16),
            pltpu.VMEM((R, D), BF16),
            pltpu.VMEM((D, F), BF16),
            pltpu.VMEM((D, F), BF16),
            pltpu.VMEM((F, D), BF16),
            pltpu.VMEM((NG, HG, GR), U32),
            pltpu.VMEM((NG, NJ, HG, LANES), F32),
            pltpu.VMEM((NG, NJ, HG, LANES), U32),
            pltpu.VMEM((NG, HG, GR), F32),
            pltpu.VMEM((8, F), U32),
            pltpu.VMEM((4, 8, PR), U32),
            pltpu.VMEM((8, PR), U32),
            pltpu.VMEM((D, LANES), F32),
            pltpu.VMEM((NP, 8, 4 * PR), U32),
            pltpu.VMEM((NP - NV, 8, W), U32),
            pltpu.VMEM((8, (NP - NV) * PR), U32),
            *[pltpu.VMEM((2 * NJ, 8, LANES), F32)] * NV,
            pltpu.SemaphoreType.DMA((AHEAD + 3,)),
        ],
        compiler_params=pltpu.CompilerParams(vmem_limit_bytes=127 * 1024 * 1024),
    )(A_x.reshape(1, D), k_t, v_t, A_wq, A_wo, B_w1, B_w3, B_w2)
    return out.reshape(A_x.shape)
```

```python
import jax
import jax.numpy as jnp
from jax import lax
import jax.experimental.pallas as pl
import jax.experimental.pallas.tpu as pltpu

BF16 = jnp.bfloat16
F32 = jnp.float32
U32 = jnp.uint32

HQ, DH = 32, 192
R = HQ * DH
LANES = 128
HG = 8
NG = HQ // HG
GR = HG * DH
NP = HQ // 2
PR = 2 * DH
PT = PR // LANES
EPS = 1e-5
LOG2E = 1.4426950408889634

AHEAD = 4
QC = 512

NV = 10
NQV = 8
NFV = 1
IB = 2
MT = 4
JS = 8
Q_AHEAD = 2
WO_AT = 20

MXU_TILE = 8.5
VPU_BLOCK = 136
Q_STEP = 3.6
SOFTMAX_LAT = 400
COL_LAT = 150
VPU_LAT, TIE_EVERY = 250, 2
F_LAT, F_TIE = 150, 2
DM, DM_AT = 8, 5
QPART = 20


def _layernorm(x):
    m = jnp.mean(x, axis=-1, keepdims=True)
    c = x - m
    v = jnp.mean(c * c, axis=-1, keepdims=True)
    return c / jnp.sqrt(v + EPS)


def _rnd(x):
    return x.astype(BF16).astype(F32)


def _bf(u):
    return pltpu.bitcast(u, BF16)


def _pack(x):
    return pltpu.bitcast(jnp.concatenate([x, jnp.zeros_like(x)], axis=0).astype(BF16), U32)


def _dot(a, b):
    return jnp.dot(a, b, preferred_element_type=F32)


def _lanes(i):
    return slice(i * LANES, (i + 1) * LANES)


class _Streams:
    def __init__(self, never, mxu, vpu_lat, tie_every):
        self.vpu_lat, self.tie_every = vpu_lat, tie_every
        self.never = never
        self.mxu = mxu
        self.tm, self.tv = 0, COL_LAT
        self.mxu_result = None
        self.vpu_results = []
        self.tied = -1
        self.tiles = next(mxu)

    def after_mxu(self, i, v):
        if i % DM == DM_AT and self.mxu_result is not None:
            return jnp.where(self.never, self.mxu_result, v)
        return v

    def after_vpu(self, u):
        prev = [k for k, (t, _) in enumerate(self.vpu_results) if t + self.vpu_lat <= self.tm]
        if not prev or prev[-1] < self.tied + self.tie_every:
            return _bf(u)
        self.tied = prev[-1]
        us = [pltpu.bitcast(v, U32) for v in self.vpu_results[self.tied][1]]
        while len(us) > 1:
            us = [a | b for a, b in zip(us[0::2], us[1::2])] + us[len(us) // 2 * 2:]
        first = jnp.where(self.never, us[0], u[:, 0:LANES])
        if u.shape[1] == LANES:
            return _bf(first)
        return _bf(jnp.concatenate([first, u[:, LANES:]], axis=1))

    def vpu_done(self, values):
        self.vpu_results.append((self.tv, values))

    def mxu_step(self):
        tiles, self.tiles = self.tiles, next(self.mxu, None)
        self.tm += MXU_TILE * tiles

    def vpu_run(self, task, cost):
        for steps in task:
            while self.tiles and self.tm <= self.tv:
                self.mxu_step()
            self.tv += cost * steps

    def finish(self):
        while self.tiles:
            self.mxu_step()

    def chain(self, lhs, rhs, n, step):
        acc = None
        for k in range(0, n, step):
            m = min(step, n - k)
            yield MT * m / step
            y = _dot(self.after_vpu(lhs(k, m)), rhs(k, m))[0:8]
            acc = y if acc is None else acc + y
            self.mxu_result = acc[:, 0:LANES]
        return acc


def _make_kernel(D, F, SK, W):
    NJ = W // LANES
    ND = D // LANES
    cexp = DH ** -0.5 * LOG2E

    def kernel(x_hbm, k_hbm, v_hbm, wq_hbm, wo_hbm, w1_hbm, w3_hbm, w2_hbm, o_ref,
               xb, kb, vb, wq, wo, w1, w3, w2,
               gq_ref, gs_ref, gp_ref, gacc_ref, act_ref,
               qm_ref, om_ref, hc_ref, lhs_ref, pm_ref, ob_ref, *rest):
        pv_refs, sems = rest[:NV], rest[NV]

        def k_copy(j):
            return pltpu.make_async_copy(
                k_hbm.at[:, pl.ds(SK - W + j * LANES, LANES)], kb.at[j], sems.at[j % AHEAD])

        def v_copy(j):
            return pltpu.make_async_copy(
                v_hbm.at[:, pl.ds(SK - W + j * LANES, LANES)], vb.at[j], sems.at[j % AHEAD])

        def rows_copy(src, dst, r0, n, sem):
            return pltpu.make_async_copy(
                src.at[pl.ds(r0, n)], dst.at[pl.ds(r0, n)], sems.at[sem])

        def start(copy, j, q):
            copy(j).start(priority=q)

        def start_both(copies):
            for q, c in enumerate(copies):
                c.start(priority=q)

        def wait(copies):
            for c in copies:
                c.wait()

        x_copy = pltpu.make_async_copy(x_hbm, xb, sems.at[AHEAD + 2])
        wq_copy = [rows_copy(wq_hbm, wq, q * D // 2, D // 2, AHEAD + q) for q in range(2)]
        wo_copy = [rows_copy(wo_hbm, wo, q * R // 2, R // 2, AHEAD + q) for q in range(2)]
        w13_copy = [pltpu.make_async_copy(w1_hbm, w1, sems.at[0]),
                    pltpu.make_async_copy(w3_hbm, w3, sems.at[1])]
        w2_copy = [[rows_copy(w2_hbm, w2, n * QC + q * QC // 2, QC // 2, sem + q)
                    for q in range(2)] for n, sem in enumerate((2, AHEAD, 0))]

        x_copy.start()
        start_both(wq_copy)
        for j in range(AHEAD):
            start(k_copy, j, j % 2)

        kbu = kb.bitcast(U32)
        vbu = vb.bitcast(U32)

        sub = lax.broadcasted_iota(jnp.int32, (8, PR), 0)
        lane = lax.broadcasted_iota(jnp.int32, (8, PR), 1)
        half = jnp.where(lane < DH, jnp.uint32(0x0000FFFF), jnp.uint32(0xFFFF0000))
        for ph in range(4):
            qm_ref[ph] = jnp.where(sub == ph, half, jnp.uint32(0))
        om_ref[...] = half

        def normed(x):
            return jnp.broadcast_to(_layernorm(x), (16, D)).astype(BF16)

        def normed2(x):
            c = x - jnp.mean(x, axis=-1, keepdims=True)
            rstd = 1.0 / jnp.sqrt(jnp.mean(c * c, axis=-1, keepdims=True) + EPS)
            h = jnp.broadcast_to(c, (16, D)).astype(BF16)
            hf = h[0:8].astype(F32)
            for k in range(ND):
                hc_ref[_lanes(k), :] = jnp.concatenate([hf[:, _lanes(k)]] * (LANES // 8), axis=0).T
            return pltpu.bitcast(h, U32), rstd

        def mxu_project(sm, hu, slabs):
            return sm().chain(
                lambda k, m: hu[:, _lanes(k)],
                lambda k, m: jnp.concatenate(
                    [w[_lanes(k), c0:c0 + 2 * LANES] for w, c0 in slabs], axis=1),
                ND, 1)

        def vpu_project(sm, slabs):
            accs = [None] * (2 * len(slabs))
            for i in range(D // 8):
                if i % JS == 0:
                    yield JS
                hi = sm().after_mxu(i, hc_ref[8 * i:8 * i + 8, :])
                for n, (w, c0) in enumerate(slabs):
                    wf = w[8 * i:8 * i + 8, c0:c0 + 2 * LANES].astype(F32)
                    for u in range(2):
                        t = wf[:, _lanes(u)] * hi
                        accs[2 * n + u] = t if i == 0 else accs[2 * n + u] + t
                if i % QPART == QPART - 1:
                    sm().vpu_done(list(accs))
            for shift in (4, 2, 1):
                accs = [a + pltpu.roll(a, shift, 0) for a in accs]
            return jnp.concatenate(accs, axis=1)

        def attention1(x):
            row = lax.broadcasted_iota(jnp.int32, (HG, GR), 0)
            col = lax.broadcasted_iota(jnp.int32, (HG, GR), 1)
            diag = (col >= row * DH) & (col < (row + 1) * DH)
            h = normed(x)
            wait(wq_copy)

            @pl.loop(0, NG)
            def _(g):
                q = _dot(h, wq[:, pl.ds(pl.multiple_of(g * GR, GR), GR)])[0:HG]
                gq_ref[g] = _pack(jnp.where(diag, q, 0.0))

            def rows(g):
                return pl.ds(pl.multiple_of(g * (GR // 2), GR // 2), GR // 2)

            @pl.loop(0, NJ, step=2)
            def _(j0):
                k_copy(j0).wait()
                k_copy(j0 + 1).wait()

                @pl.when(j0 + AHEAD < NJ)
                def _():
                    for q in range(2):
                        start(k_copy, j0 + q + AHEAD, q)

                @pl.when(j0 + AHEAD >= NJ)
                def _():
                    for q in range(2):
                        start(v_copy, j0 + q + AHEAD - NJ, q)

                @pl.loop(0, 2 * NG)
                def _(i):
                    j, g = j0 + i // NG, i % NG
                    gs_ref[g, j] = _dot(_bf(gq_ref[g]), _bf(kbu[j, rows(g), :]))[0:HG]

            @pl.loop(0, NG)
            def _(g):
                s = gs_ref[g]
                m = jnp.max(jnp.max(s, axis=0), axis=-1, keepdims=True)
                e = jnp.exp2((s - m[None]) * cexp)
                l = jnp.sum(jnp.sum(e, axis=0), axis=-1, keepdims=True)
                p = e * (1.0 / l)[None]
                gp_ref[g] = pltpu.bitcast(
                    jnp.concatenate([p, jnp.zeros_like(p)], axis=1).astype(BF16), U32)
                gacc_ref[g] = jnp.zeros((HG, GR), F32)

            @pl.loop(0, NJ)
            def _(j):
                v_copy(j).wait()

                for q in range(2):
                    @pl.when((j + AHEAD < NJ) & (j % 2 == q))
                    def _():
                        start(v_copy, j + AHEAD, q)

                @pl.when(j + AHEAD == NJ + 1)
                def _():
                    start_both(wo_copy)

                for g in range(NG):
                    vt = _bf(vbu[j, g * GR // 2:(g + 1) * GR // 2, :])
                    o = lax.dot_general(_bf(gp_ref[g, j]), vt, (((1,), (1,)), ((), ())),
                                        preferred_element_type=F32)
                    gacc_ref[g] += o[0:HG]
                    for t in range(GR // LANES):
                        r0 = g * GR + t * LANES
                        if r0 >= NV * PR:
                            vbu[j, r0 // 2:(r0 + LANES) // 2, :] = pltpu.bitcast(
                                vt[_lanes(t)].T, U32)

            start_both(w13_copy)

            @pl.loop(0, NG)
            def _(g):
                gq_ref[g] = _pack(jnp.where(diag, gacc_ref[g], 0.0))

            wait(wo_copy)

            def project(g, y):
                r = pl.ds(pl.multiple_of(g * GR, GR), GR)
                return y + _dot(_bf(gq_ref[g]), wo[r, :])[0:HG]

            y = lax.fori_loop(0, NG, project, jnp.zeros((HG, D), F32))
            start_both(w2_copy[0])
            return jnp.sum(y, axis=0, keepdims=True)

        def ffn1(x):
            h = normed(x)
            wait(w13_copy)
            start_both(w2_copy[1])

            @pl.loop(0, F // QC)
            def _(n):
                cols = pl.ds(pl.multiple_of(n * QC, QC), QC)
                gate = _dot(h, w1[:, cols])
                up = _dot(h, w3[:, cols])
                act_ref[:, cols] = pltpu.bitcast(
                    (gate * jax.nn.sigmoid(gate) * up).astype(BF16), U32)

            start_both(w2_copy[2])
            y = 0.0
            for n in range(F // QC):
                wait(w2_copy[n])
                y = y + _dot(_bf(act_ref[:, n * QC:(n + 1) * QC]), w2[n * QC:(n + 1) * QC, :])[0:1]
            return y

        def ffn2(x):
            hu, rstd = normed2(x)
            sm = lambda: streams
            nm = F // (2 * LANES) - NFV
            out = []

            def gated(project, n):
                c0 = 2 * LANES * n
                y = rstd * (yield from project([(w1, c0), (w3, c0)]))
                gate, up = y[:, 0:2 * LANES], y[:, 2 * LANES:]
                act_ref[:, c0:c0 + 2 * LANES] = _pack(gate * jax.nn.sigmoid(gate) * up)

            def down(k0, k1):
                for c in range(ND):
                    out.append((yield from streams.chain(
                        lambda k, m: act_ref[:, (k0 + k) * LANES:(k0 + k + m) * LANES],
                        lambda k, m: w2[(k0 + k) * LANES:(k0 + k + m) * LANES, _lanes(c)],
                        k1 - k0, MT)))

            def mxu_stream():
                yield 0.1
                for n in range(nm):
                    yield from gated(lambda slabs: mxu_project(sm, hu, slabs), n)
                yield from down(0, 2 * nm)

            streams = _Streams(om_ref[:, 0:LANES] == jnp.uint32(0), mxu_stream(), F_LAT, F_TIE)
            for n in range(nm, nm + NFV):
                streams.vpu_run(gated(lambda slabs: vpu_project(sm, slabs), n), Q_STEP)
            streams.finish()
            for _ in down(2 * nm, F // LANES):
                pass
            return jnp.concatenate(
                [sum(out[c + ND::ND], out[c])[0:1] for c in range(ND)], axis=1)

        def attention2(x):
            hu, rstd = normed2(x)
            sm = lambda: streams
            out = [None] * ND
            st = {}

            def accumulate(c, y):
                out[c] = y if out[c] is None else out[c] + y

            def q_chunk(project, n):
                q = yield from project([(wq, n * QC), (wq, n * QC + QC // 2)])
                qu = _pack(q * rstd)
                for i in range(QC // LANES):
                    p, t = divmod(n * QC // LANES + i, PT)
                    st["q", p, t] = True
                    for ph in range(4):
                        lhs_ref[p, :, _lanes(ph * PT + t)] = (
                            qu[:, _lanes(i)] & qm_ref[ph, :, _lanes(t)])

            def tile(ref, j, t):
                return _bf(ref[j, t * LANES // 2:(t + 1) * LANES // 2, :])

            def qk(p):
                assert all(("q", p, t) in st for t in range(PT))
                ss = []
                for jo in range(NJ // 4):
                    ss.append((yield from streams.chain(
                        lambda k, m: lhs_ref[p, :, k * LANES:(k + m) * LANES],
                        lambda k, m: jnp.concatenate(
                            [tile(kbu, 4 * jo + i // PT, p * PT + i % PT)
                             for i in range(k, k + m)], axis=0),
                        4 * PT, MT)))
                softmax(p, ss)
                st["ready", p] = streams.tm + SOFTMAX_LAT

            def softmax(p, ss):
                m = ss[0]
                for s in ss[1:]:
                    m = jnp.maximum(m, s)
                m = jnp.maximum(m, pltpu.roll(m, 4, 0))
                m = jnp.maximum(m, pltpu.roll(m, 2, 0))
                m = jnp.max(m, axis=-1, keepdims=True)
                es = [jnp.exp2((s - m) * cexp) for s in ss]
                l = sum(es[1:], es[0])
                l = l + pltpu.roll(l, 4, 0)
                l = l + pltpu.roll(l, 2, 0)
                st["inv", p] = 1.0 / jnp.sum(l, axis=-1, keepdims=True)
                for jo, e in enumerate(es):
                    if p < NV:
                        for sl in range(8):
                            pv_refs[p][(sl % 2) * NJ + 4 * jo + sl // 2] = jnp.broadcast_to(
                                e[sl:sl + 1], (8, LANES))
                    else:
                        eu = _pack(e)
                        for ph in range(4):
                            own = qm_ref[ph, :, 0:LANES] != jnp.uint32(0)
                            pm_ref[p - NV, :, _lanes(4 * jo + ph)] = jnp.where(
                                own, eu, jnp.uint32(0))

            def mxu_pv(p, t):
                o = yield from streams.chain(
                    lambda k, m: pm_ref[p - NV, :, k * LANES:(k + m) * LANES],
                    lambda k, m: jnp.concatenate(
                        [tile(vbu, i, p * PT + t) for i in range(k, k + m)], axis=0),
                    NJ, MT)
                ob_ref[:, _lanes((p - NV) * PT + t)] = (
                    _pack(o * st["inv", p]) & om_ref[:, _lanes(t)])

            def mxu_wo(c):
                st["y", c] = yield from streams.chain(
                    lambda k, m: ob_ref[:, k * LANES:(k + m) * LANES],
                    lambda k, m: wo[NV * PR + k * LANES:NV * PR + (k + m) * LANES, _lanes(c)],
                    (NP - NV) * PT, MT)

            def vpu_wo():
                if "os" not in st:
                    return
                r0, os_ = st.pop("os")
                for c in range(ND):
                    wf = wo[r0:r0 + 16 * IB, _lanes(c)].astype(F32)
                    y = None
                    for a in range(2 * IB):
                        t = wf[8 * a:8 * a + 8] * os_[a]
                        y = t if y is None else y + t
                    accumulate(c, y)

            def vpu_pv(p, hd, blk):
                r0 = p * PR + hd * DH + blk * 16 * IB
                base = hd * NJ
                accs = [None] * (2 * IB)
                for j in range(NJ):
                    if j % JS == 0:
                        yield JS
                    if j == WO_AT:
                        vpu_wo()
                    pj = streams.after_mxu(j, pv_refs[p][base + j])
                    vf = vb[j, r0:r0 + 16 * IB, :].astype(F32)
                    for a in range(2 * IB):
                        t = vf[8 * a:8 * a + 8] * pj
                        accs[a] = t if accs[a] is None else accs[a] + t
                if blk == 0:
                    st["scale"] = jnp.broadcast_to(st["inv", p][hd:hd + 1], (8, 1))
                st["os"] = (r0, [jnp.sum(a, axis=-1, keepdims=True) * st["scale"] for a in accs])
                streams.vpu_done(accs + [y for y in out if y is not None])

            def mxu_stream():
                yield 0.1
                nq = 0
                for p in range(NP):
                    while nq < R // QC - NQV and nq * QC < (p + Q_AHEAD if p else 1) * PR:
                        yield from q_chunk(lambda slabs: mxu_project(sm, hu, slabs), nq)
                        nq += 1
                    yield from qk(p)
                    if p > NV:
                        for t in range(PT):
                            yield from mxu_pv(p - 1, t)
                for t in range(PT):
                    yield from mxu_pv(NP - 1, t)
                for c in range(ND):
                    yield from mxu_wo(c)

            streams = _Streams(om_ref[:, 0:LANES] == jnp.uint32(0), mxu_stream(), VPU_LAT, TIE_EVERY)
            for n in range(R // QC - NQV, R // QC):
                streams.vpu_run(q_chunk(lambda slabs: vpu_project(sm, slabs), n), Q_STEP)
            for p in range(NV):
                while ("ready", p) not in st:
                    streams.mxu_step()
                streams.tv = max(streams.tv, st["ready", p])
                for hd in range(2):
                    for blk in range(DH // (16 * IB)):
                        streams.vpu_run(vpu_pv(p, hd, blk), VPU_BLOCK / NJ)
            vpu_wo()
            streams.finish()
            return jnp.concatenate(
                [jnp.sum(out[c] + st["y", c], axis=0, keepdims=True) for c in range(ND)], axis=1)

        x_copy.wait()
        x = xb[...].astype(F32)
        x = _rnd(x + _rnd(attention1(x)))
        x = _rnd(x + _rnd(ffn1(x)))
        x = _rnd(x + _rnd(attention2(x)))
        x = _rnd(x + _rnd(ffn2(x)))
        o_ref[...] = x.astype(o_ref.dtype)

    return kernel


@jax.jit
def pallas_interleave_layers__sliding_block_cached__glu_gated_swiglu__decode_kernel(
    A_x: jax.Array,
    A_k_cache: jax.Array,
    A_v_cache: jax.Array,
    A_wq: jax.Array,
    A_wo: jax.Array,
    B_x: jax.Array,
    B_w1: jax.Array,
    B_w3: jax.Array,
    B_w2: jax.Array,
):
    del B_x
    D = A_x.shape[-1]
    F = B_w1.shape[-1]
    SK = A_k_cache.shape[2]
    W = min(4096, max(256, SK // 4))
    NJ = W // LANES
    ND = D // LANES

    k_t = jnp.swapaxes(A_k_cache, 2, 3).reshape(R, SK)
    v_t = jnp.swapaxes(A_v_cache, 2, 3).reshape(R, SK)

    hbm = pl.BlockSpec(memory_space=pl.ANY)
    out = pl.pallas_call(
        _make_kernel(D, F, SK, W),
        out_shape=jax.ShapeDtypeStruct((1, D), A_x.dtype),
        in_specs=[hbm] * 8,
        out_specs=pl.BlockSpec(memory_space=pltpu.VMEM),
        scratch_shapes=[
            pltpu.VMEM((1, D), BF16),
            pltpu.VMEM((NJ, R, LANES), BF16),
            pltpu.VMEM((NJ, R, LANES), BF16),
            pltpu.VMEM((D, R), BF16),
            pltpu.VMEM((R, D), BF16),
            pltpu.VMEM((D, F), BF16),
            pltpu.VMEM((D, F), BF16),
            pltpu.VMEM((F, D), BF16),
            pltpu.VMEM((NG, HG, GR), U32),
            pltpu.VMEM((NG, NJ, HG, LANES), F32),
            pltpu.VMEM((NG, NJ, HG, LANES), U32),
            pltpu.VMEM((NG, HG, GR), F32),
            pltpu.VMEM((8, F), U32),
            pltpu.VMEM((4, 8, PR), U32),
            pltpu.VMEM((8, PR), U32),
            pltpu.VMEM((D, LANES), F32),
            pltpu.VMEM((NP, 8, 4 * PR), U32),
            pltpu.VMEM((NP - NV, 8, W), U32),
            pltpu.VMEM((8, (NP - NV) * PR), U32),
            *[pltpu.VMEM((2 * NJ, 8, LANES), F32)] * NV,
            pltpu.SemaphoreType.DMA((AHEAD + 3,)),
        ],
        compiler_params=pltpu.CompilerParams(vmem_limit_bytes=127 * 1024 * 1024),
    )(A_x.reshape(1, D), k_t, v_t, A_wq, A_wo, B_w1, B_w3, B_w2)
    return out.reshape(A_x.shape)
```
